```python
import jax
import jax.numpy as jnp

def _softmax(x, axis=-1):
    return jax.nn.softmax(x, axis=axis)
def _gelu(x):
    return jax.nn.gelu(x, approximate=True)
def _silu(x):
    return jax.nn.silu(x)
def _sigmoid(x):
    return jax.nn.sigmoid(x)
def _layernorm(x, axis=-1, eps=1e-5):
    m = jnp.mean(x, axis=axis, keepdims=True)
    v = jnp.var(x, axis=axis, keepdims=True)
    return (x - m) / jnp.sqrt(v + eps)
def _scatter_add(tgt, idx, src, axis=0):
    return tgt.at[idx].add(src)
def _segment_sum(src, seg, n):
    return jax.ops.segment_sum(src, seg, n)
class _Rng:
    def __init__(self, key):
        self._k = key
    def _next(self):
        self._k, sub = jax.random.split(self._k)
        return sub
    def normal(self, shape):
        return jax.random.normal(self._next(), shape, dtype=jnp.bfloat16)
    def randint(self, lo, hi, shape):
        return jax.random.randint(self._next(), shape, lo, hi, dtype=jnp.int32)
    def uniform(self, shape, lo=0.0, hi=1.0):
        return jax.random.uniform(self._next(), shape, jnp.bfloat16, lo, hi)
    def permutation(self, n):
        return jax.random.permutation(self._next(), n)


kernel_name = 'standalone__adm_resblock__diffusion'

def setup_inputs():
    _rng = _Rng(jax.random.key(int.from_bytes(__import__("os").urandom(4), "little")))
    _w = (lambda a: (lambda t: t.astype(jnp.bfloat16) if jnp.issubdtype(t.dtype, jnp.floating) else t)(jnp.asarray(a)))
    B, C, HW, E = 2, 512, 64, 1152
    sc = (9.0 * C) ** -0.5
    return {
        "x": _w((lambda *s: _rng.normal(s) * 0.05)(B, C, HW, HW)),
        "t_emb": _w((lambda *s: _rng.normal(s) * 0.05)(B, E)),
        "g1": _w(1.0 + 0.1 * (lambda *s: _rng.normal(s) * 0.05)(C)),
        "be1": _w(0.1 * (lambda *s: _rng.normal(s) * 0.05)(C)),
        "w1": _w((lambda *s: _rng.normal(s) * 0.05)(C, C, 3, 3) * sc),
        "w_emb": _w((lambda *s: _rng.normal(s) * 0.05)(E, C) * (E ** -0.5)),
        "g2": _w(1.0 + 0.1 * (lambda *s: _rng.normal(s) * 0.05)(C)),
        "be2": _w(0.1 * (lambda *s: _rng.normal(s) * 0.05)(C)),
        "w2": _w((lambda *s: _rng.normal(s) * 0.05)(C, C, 3, 3) * sc),
    }

def reference(x, t_emb, g1, be1, w1, w_emb, g2, be2, w2):
    B, C, H, W = x.shape
    G, eps = 4, 1e-5
    def gn(z, gamma, beta):
        zr = z.reshape(B, G, (C // G) * H * W)
        mu = zr.mean(-1).reshape(B, G, 1)
        var = ((zr - mu) ** 2).mean(-1).reshape(B, G, 1)
        zn = ((zr - mu) / jnp.sqrt(var + eps)).reshape(B, C, H, W)
        return zn * gamma.reshape(1, C, 1, 1) + beta.reshape(1, C, 1, 1)
    def conv3(z, w):
        zp = jnp.pad(z, ((0, 0), (0, 0), (1, 1), (1, 1)))
        taps = [jnp.einsum("bchw,oc->bohw", zp[:, :, i:i+H, j:j+W], w[:, :, i, j]) for i in range(3) for j in range(3)]
        out = taps[0]
        for t in taps[1:]:
            out = out + t
        return out
    h = conv3(_silu(gn(x, g1, be1)), w1)
    emb = _silu(t_emb) @ w_emb
    h = h + emb.reshape(B, C, 1, 1)
    h = conv3(_silu(gn(h, g2, be2)), w2)
    return x + h
```

```python
import functools

import jax
import jax.numpy as jnp
import numpy as np
from jax import lax
import jax.experimental.pallas as pl
import jax.experimental.pallas.tpu as pltpu

F32, BF16, U32 = jnp.float32, jnp.bfloat16, jnp.uint32

PA, PB = 1.5, 2.0 / 3.0
NA = 2.0 * PA * PA * (PA * PA - PB * PB)
NB = 2.0 * PB * PB * (PB * PB - PA * PA)
EPS = 1e-5


def _mul(x, c):
    return lax.mul(x, np.float32(c))


_add, _sub = lax.add, lax.sub


def _in_tf(d0, d1, d2, d3, d4, d5):
    p = _mul(d2, PB * PB)
    q = _mul(d2, PA * PA)
    e1 = _sub(d4, p)
    e2 = _sub(d4, q)
    r0 = _add(_sub(d0, q), e1)
    t = _mul(d3, PB * PB)
    o1 = _sub(_mul(d3, PA * PA), d1)
    o2 = _sub(t, d1)
    r5 = _sub(_sub(d5, t), o1)
    o1 = _mul(o1, PB)
    o2 = _mul(o2, PA)
    return r0, _add(e1, o1), _sub(e1, o1), _add(e2, o2), _sub(e2, o2), r5


def _out_tf(m0, m1, m2, m3, m4, m5):
    s1, d1 = _add(m1, m2), _sub(m1, m2)
    s2, d2 = _add(m3, m4), _sub(m3, m4)
    y0 = _add(_add(m0, s1), s2)
    y1 = _add(_mul(d1, PA), _mul(d2, PB))
    y2 = _add(_mul(s1, PA * PA), _mul(s2, PB * PB))
    y3 = _add(_add(_mul(d1, PA ** 3), _mul(d2, PB ** 3)), m5)
    return y0, y1, y2, y3


def _w_tf(g0, g1, g2):
    ea = _add(_mul(g0, 1.0 / NA), _mul(g2, PA * PA / NA))
    oa = _mul(g1, PA / NA)
    eb = _add(_mul(g0, 1.0 / NB), _mul(g2, PB * PB / NB))
    ob = _mul(g1, PB / NB)
    return g0, _add(ea, oa), _sub(ea, oa), _add(eb, ob), _sub(eb, ob), g2


def _lo(w):
    return lax.bitcast_convert_type(lax.shift_left(w, np.uint32(16)), F32)


def _hi(w):
    return lax.bitcast_convert_type(lax.bitwise_and(w, np.uint32(0xFFFF0000)), F32)


def _cat(a, b):
    return lax.concatenate([a, b], 0)


def _interleave(*tasks):
    done = [0] * len(tasks)
    live = [True] * len(tasks)
    while any(live):
        i = min((k for k in range(len(tasks)) if live[k]),
                key=lambda k: (done[k] + 0.5) / tasks[k][1])
        try:
            next(tasks[i][0])
            done[i] += 1
        except StopIteration:
            live[i] = False


def _kernel(x_hbm, t_ref, g1_ref, be1_ref, w1_hbm, we_hbm, g2_ref, be2_ref, w2_hbm,
            o_hbm,
            xs, ws, wes, us, vs, ms, hs, ts, os_, par, cfx, cfh,
            xsem, wsem, esem, osem):
    xw = xs.bitcast(U32)
    ow = os_.bitcast(U32)

    def x_copy(bg):
        b, g = bg // 4, bg % 4
        return pltpu.make_async_copy(
            x_hbm.at[b, :, pl.ds(g * 128, 128)], xs.at[bg], xsem.at[bg])

    def w_copies(c):
        w = w1_hbm if c < 4 else w2_hbm
        n = c % 4
        return [pltpu.make_async_copy(
            w.at[:, pl.ds(n * 128, 128), pl.ds(k * 128, 128)], ws.at[c, k], wsem.at[c])
            for k in range(4)]

    def w_wait(c):
        pltpu.make_async_copy(ws.at[c], ws.at[c], wsem.at[c]).wait()

    def o_copy(slot, bg):
        b, g = bg // 4, bg % 4
        return pltpu.make_async_copy(
            os_.at[slot], o_hbm.at[b, :, pl.ds(pl.multiple_of(g * 128, 128), 128)],
            osem.at[slot])

    e_copy = pltpu.make_async_copy(we_hbm, wes, esem)

    def finalize(s1, s2, emb, gamma, beta, cf, bg):
        inv = 1.0 / 4096.0
        m = jnp.sum(s1, axis=0, keepdims=True) * inv
        v = jnp.maximum(jnp.sum(s2, axis=0, keepdims=True) * inv - m * m, 0.0)
        if emb is not None:
            m = m + emb
        mu = jnp.sum(m, axis=1, keepdims=True) * (1.0 / 128.0)
        dm = m - mu
        var = jnp.sum(v + dm * dm, axis=1, keepdims=True) * (1.0 / 128.0)
        sc = lax.rsqrt(var + EPS) * gamma * 0.5
        sh = (0.5 * beta) - (mu if emb is None else mu - emb) * sc
        cf[bg, 0] = jnp.broadcast_to(sc, (16, 128))
        cf[bg, 1] = jnp.broadcast_to(sh, (16, 128))

    NX = 33

    def x_stats(bg):
        g = bg % 4
        s1 = s2 = None
        for r in range(32):
            w = xw[bg, pl.ds(r * 64, 64), :]
            lo, hi = _lo(w), _hi(w)
            a = _add(lo, hi)
            q = _add(lax.mul(lo, lo), lax.mul(hi, hi))
            a = _add(a[:32], a[32:])
            q = _add(q[:32], q[32:])
            a = _add(a[:16], a[16:])
            q = _add(q[:16], q[16:])
            s1 = a if s1 is None else _add(s1, a)
            s2 = q if s2 is None else _add(s2, q)
            yield
        finalize(s1, s2, None, par[0, g], par[1, g], cfx, bg)
        yield

    NA_ = 64 + 96

    def in_stage(src_x, bg, vb):
        g = bg % 4
        cf = cfx if src_x else cfh
        sc, sh = cf[bg, 0], cf[bg, 1]
        sub = lax.broadcasted_iota(jnp.int32, (8, 128), 0)
        first, last = sub == 0, sub == 7
        zero = jnp.zeros((8, 128), F32)

        def row(h):
            if src_x:
                w = [xw[bg, pl.ds(h * 32 + k, 8, stride=4), :] for k in range(4)]
                w02, w13 = _cat(w[0], w[2]), _cat(w[1], w[3])
                y = [_lo(w02), _hi(w02), _lo(w13), _hi(w13)]
            else:
                y = [hs[bg, h, j] for j in range(4)]
            a = []
            for yj in y:
                u = _add(lax.mul(yj, sc), sh)
                a.append(_add(u, lax.mul(u, lax.tanh(u))))
            left = lax.select(first, zero, pltpu.roll(a[3][8:], 1, 0))
            right = lax.select(last, zero, pltpu.roll(a[0][:8], 7, 0))
            r = _in_tf(_cat(left, a[3][:8]), a[0], a[1], a[2], a[3], _cat(a[0][8:], right))
            for jj in range(6):
                ts[h + 1, jj] = r[jj]

        def col(th, jj):
            r = _in_tf(*[ts[4 * th + i, jj] for i in range(6)])
            for ii in range(6):
                vs[vb, ii * 6 + jj, g, pl.ds(th * 8, 8), :] = pltpu.bitcast(
                    r[ii].astype(BF16), U32)

        h = 0
        for th in range(16):
            while h < min(64, 4 * th + 9):
                row(h)
                h += 1
                yield
            for jj in range(6):
                col(th, jj)
                yield

    NC_ = 33

    def out_tile(mb, th, e):
        rows = pl.ds(th * 16 + e * 8, 8)
        z = [_out_tf(*[ms[mb, i * 6 + j, rows, :] for j in range(6)]) for i in range(6)]
        return [_out_tf(*[z[i][q] for i in range(6)]) for q in range(4)]

    def out_stage1(mb, bg):
        b, g = bg // 4, bg % 4
        s1 = s2 = None
        for th in range(16):
            for e in range(2):
                y = out_tile(mb, th, e)
                for q in range(4):
                    for p in range(4):
                        hs[bg, 4 * th + p, q, pl.ds(e * 8, 8), :] = y[q][p]
                    a = _add(_add(y[q][0], y[q][1]), _add(y[q][2], y[q][3]))
                    sq = [lax.mul(v, v) for v in y[q]]
                    c = _add(_add(sq[0], sq[1]), _add(sq[2], sq[3]))
                    s1 = a if s1 is None else _add(s1, a)
                    s2 = c if s2 is None else _add(s2, c)
                yield
        finalize(s1, s2, par[4 + b, g], par[2, g], par[3, g], cfh, bg)
        yield

    def out_stage2(mb, bg, slot):
        for th in range(16):
            for e in range(2):
                y = out_tile(mb, th, e)
                for p in range(4):
                    for kq in range(2):
                        rows = pl.ds((4 * th + p) * 32 + 2 * e + kq, 8, stride=4)
                        w = xw[bg, rows, :]
                        v = _cat(_add(y[2 * kq][p], _lo(w)), _add(y[2 * kq + 1][p], _hi(w)))
                        v = lax.bitcast_convert_type(v.astype(BF16).astype(F32), U32)
                        ow[slot, rows, :] = lax.bitwise_or(
                            lax.shift_right_logical(v[:8], np.uint32(16)), v[8:])
                yield
        yield

    NU = 32

    def w_stage(c):
        for k in range(4):
            for r in range(8):
                g = [ws[c, k, t, pl.ds(r * 16, 16), :].astype(F32) for t in range(9)]
                t1 = [_w_tf(g[3 * i], g[3 * i + 1], g[3 * i + 2]) for i in range(3)]
                for jj in range(6):
                    u = _w_tf(t1[0][jj], t1[1][jj], t1[2][jj])
                    for ii in range(6):
                        us[c, ii * 6 + jj, k, pl.ds(r * 8, 8), :] = pltpu.bitcast(
                            u[ii].astype(BF16), U32)
                yield

    NB_ = 37

    def mm_stage(vb, c, mb):
        for ij in range(36):
            lhs = lax.concatenate([pltpu.bitcast(vs[vb, ij, k], BF16) for k in range(4)], 1)
            rhs = lax.concatenate([pltpu.bitcast(us[c, ij, k], BF16) for k in range(4)], 1)
            ms[mb, ij] = lax.dot_general(lhs, rhs, (((1,), (1,)), ((), ())),
                                         preferred_element_type=F32)
            yield

    def run(gen):
        for _ in gen:
            pass

    for bg in range(4):
        x_copy(bg).start()
    for cp in w_copies(0):
        cp.start()
    for i, ref in enumerate((g1_ref, be1_ref, g2_ref, be2_ref)):
        v = ref[...].astype(F32)
        for g in range(4):
            par[i, g] = v[:, g * 128:(g + 1) * 128]
    ts[0] = jnp.zeros((6, 16, 128), F32)
    ts[65] = jnp.zeros((6, 16, 128), F32)

    def pro(g, carry):
        pltpu.make_async_copy(xs.at[g], xs.at[g], xsem.at[g]).wait()

        @pl.when(g == 1)
        def _():
            x_copy(4).start()
            for cp in w_copies(1):
                cp.start()
            e_copy.start()

        run(x_stats(g))
        run(in_stage(True, g, 0))
        return carry

    lax.fori_loop(0, 4, pro, 0)
    for bg in range(5, 8):
        x_copy(bg).start()
    for c in range(2, 8):
        for cp in w_copies(c):
            cp.start()
    w_wait(0)
    run(w_stage(0))
    e_copy.wait()
    t = t_ref[...].astype(F32)
    t = (t * jax.nn.sigmoid(t)).astype(BF16)
    emb = jnp.dot(t, wes[...], preferred_element_type=F32)
    for b in range(2):
        for g in range(4):
            par[4 + b, g] = emb[b:b + 1, g * 128:(g + 1) * 128]

    def chain(*gens):
        for gen in gens:
            yield from gen

    def step(s, kind, do_c, do_a, do_u):
        u = s // 4
        tasks = [(mm_stage(u % 2, (u // 2) * 4 + s % 4, s % 2), NB_)]
        if do_c == 1:
            tasks.append((out_stage1((s - 1) % 2, s - 1), NC_))
        elif do_c == 2:
            tasks.append((out_stage2((s - 1) % 2, s - 9, (s - 1) % 2), NC_))
        if do_a == 'x':
            tasks.append((chain(x_stats(s + 4), in_stage(True, s + 4, 1)), NX + NA_))
        elif do_a == 'h':
            tasks.append((in_stage(False, s - 4, (u + 1) % 2), NA_))
        if do_u:
            tasks.append((w_stage(s + 1), NU))
        _interleave(*tasks)

    def x_wait(bg):
        pltpu.make_async_copy(xs.at[bg], xs.at[bg], xsem.at[bg]).wait()

    x_wait(4)
    w_wait(1)
    step(0, 0, 0, 'x', True)

    def loop1(s, carry):
        x_wait(s + 4)
        w_wait(s + 1)
        step(s, 0, 1, 'x', True)
        return carry

    lax.fori_loop(1, 4, loop1, 0)

    def loop2(s, carry):
        w_wait(s + 1)
        step(s, 0, 1, 'h', True)
        return carry

    lax.fori_loop(4, 7, loop2, 0)

    def loop3(s, carry):
        step(s, 0, 1, 'h', False)
        return carry

    lax.fori_loop(7, 9, loop3, 0)

    def mk(do_a):
        def loop(s, carry):
            @pl.when(s >= 11)
            def _():
                o_copy((s - 1) % 2, s - 11).wait()
            step(s, 0, 2, do_a, False)
            o_copy((s - 1) % 2, s - 9).start()
            return carry
        return loop

    lax.fori_loop(9, 12, mk('h'), 0)
    lax.fori_loop(12, 16, mk(None), 0)
    o_copy(1, 5).wait()
    run(out_stage2(1, 7, 1))
    o_copy(1, 7).start()
    o_copy(0, 6).wait()
    o_copy(1, 7).wait()


@jax.jit
def pallas_standalone__adm_resblock__diffusion_kernel(
        x, t_emb, g1, be1, w1, w_emb, g2, be2, w2):
    B, C, H, W = x.shape
    E = t_emb.shape[1]
    assert (B, C, H, W) == (2, 512, 64, 64)
    xt = x.transpose(0, 2, 3, 1).reshape(B, H * W, C)
    w1t = w1.transpose(2, 3, 0, 1).reshape(9, C, C)
    w2t = w2.transpose(2, 3, 0, 1).reshape(9, C, C)
    hbm = pl.BlockSpec(memory_space=pl.ANY)
    vm = pl.BlockSpec(memory_space=pltpu.VMEM)
    r = lambda a: a.reshape(1, C)
    out = pl.pallas_call(
        _kernel,
        out_shape=jax.ShapeDtypeStruct((B, H * W, C), x.dtype),
        in_specs=[hbm, vm, vm, vm, hbm, hbm, vm, vm, hbm],
        out_specs=hbm,
        scratch_shapes=[
            pltpu.VMEM((8, 4096, 128), BF16),
            pltpu.VMEM((8, 4, 9, 128, 128), BF16),
            pltpu.VMEM((E, C), BF16),
            pltpu.VMEM((8, 36, 4, 64, 128), U32),
            pltpu.VMEM((2, 36, 4, 128, 128), U32),
            pltpu.VMEM((2, 36, 256, 128), F32),
            pltpu.VMEM((8, 64, 4, 16, 128), F32),
            pltpu.VMEM((66, 6, 16, 128), F32),
            pltpu.VMEM((2, 4096, 128), BF16),
            pltpu.VMEM((6, 4, 1, 128), F32),
            pltpu.VMEM((8, 2, 16, 128), F32),
            pltpu.VMEM((8, 2, 16, 128), F32),
            pltpu.SemaphoreType.DMA((8,)),
            pltpu.SemaphoreType.DMA((8,)),
            pltpu.SemaphoreType.DMA(()),
            pltpu.SemaphoreType.DMA((2,)),
        ],
        compiler_params=pltpu.CompilerParams(vmem_limit_bytes=124 * 2 ** 20),
        name="resblock",
    )(xt, t_emb, r(g1), r(be1), w1t, w_emb, r(g2), r(be2), w2t)
    return out.reshape(B, H, W, C).transpose(0, 3, 1, 2)
```

```python
import jax
import jax.numpy as jnp
import numpy as np
from jax import lax
import jax.experimental.pallas as pl
import jax.experimental.pallas.tpu as pltpu

F32, BF16, U32 = jnp.float32, jnp.bfloat16, jnp.uint32

PA, PB = 1.5, 2.0 / 3.0
NA = 2.0 * PA * PA * (PA * PA - PB * PB)
NB = 2.0 * PB * PB * (PB * PB - PA * PA)
EPS = 1e-5


def _mul(x, c):
    return lax.mul(x, np.float32(c))


_add, _sub = lax.add, lax.sub


def _in_tf(d0, d1, d2, d3, d4, d5):
    p = _mul(d2, PB * PB)
    q = _mul(d2, PA * PA)
    e1 = _sub(d4, p)
    e2 = _sub(d4, q)
    r0 = _add(_sub(d0, q), e1)
    t = _mul(d3, PB * PB)
    o1 = _sub(_mul(d3, PA * PA), d1)
    o2 = _sub(t, d1)
    r5 = _sub(_sub(d5, t), o1)
    o1 = _mul(o1, PB)
    o2 = _mul(o2, PA)
    return r0, _add(e1, o1), _sub(e1, o1), _add(e2, o2), _sub(e2, o2), r5


def _out_tf(m0, m1, m2, m3, m4, m5):
    s1, d1 = _add(m1, m2), _sub(m1, m2)
    s2, d2 = _add(m3, m4), _sub(m3, m4)
    y0 = _add(_add(m0, s1), s2)
    y1 = _add(_mul(d1, PA), _mul(d2, PB))
    y2 = _add(_mul(s1, PA * PA), _mul(s2, PB * PB))
    y3 = _add(_add(_mul(d1, PA ** 3), _mul(d2, PB ** 3)), m5)
    return y0, y1, y2, y3


def _w_eo(g0, g1, g2):
    ea = _add(_mul(g0, 1.0 / NA), _mul(g2, PA * PA / NA))
    oa = _mul(g1, PA / NA)
    eb = _add(_mul(g0, 1.0 / NB), _mul(g2, PB * PB / NB))
    ob = _mul(g1, PB / NB)
    return ea, oa, eb, ob


def _w_tf(g0, g1, g2):
    ea, oa, eb, ob = _w_eo(g0, g1, g2)
    return g0, _add(ea, oa), _sub(ea, oa), _add(eb, ob), _sub(eb, ob), g2


def _lo(w):
    return lax.bitcast_convert_type(lax.shift_left(w, np.uint32(16)), F32)


def _hi(w):
    return lax.bitcast_convert_type(lax.bitwise_and(w, np.uint32(0xFFFF0000)), F32)


def _cat(a, b):
    return lax.concatenate([a, b], 0)


def _merge(tasks):
    done = [0] * len(tasks)
    live = list(range(len(tasks)))
    while live:
        i = min(live, key=lambda k: done[k] / tasks[k][1])
        while True:
            item = next(tasks[i][0], None)
            if item is None:
                live.remove(i)
                assert done[i] == tasks[i][1], (i, done[i], tasks[i][1])
                break
            done[i] += item[0]
            yield item
            if item[2]:
                break


def _chain(*gens):
    for gen in gens:
        yield from gen


def _run(gen):
    for _ in gen:
        pass


def _kernel(x_hbm, t_ref, g1_ref, be1_ref, w1_hbm, we_hbm, g2_ref, be2_ref, w2_hbm,
            o_hbm,
            xs, ws, wes, us, vs, ms, hs, ts, os_, par, cf,
            xsem, wsem, esem, osem):
    xw = xs.bitcast(U32)
    ow = os_.bitcast(U32)
    uw = us.bitcast(U32)
    vw = vs.bitcast(U32)

    def x_copy(bg):
        b, g = bg // 4, bg % 4
        return pltpu.make_async_copy(
            x_hbm.at[b, :, pl.ds(g * 128, 128)], xs.at[bg], xsem.at[bg])

    def w_start(c):
        w = w1_hbm if c < 4 else w2_hbm
        n = c % 4
        for k in range(4):
            pltpu.make_async_copy(
                w.at[:, pl.ds(n * 128, 128), pl.ds(k * 128, 128)], ws.at[c, k],
                wsem.at[c]).start()

    def w_wait(c):
        pltpu.make_async_copy(ws.at[c], ws.at[c], wsem.at[c]).wait()

    def x_wait(bg):
        pltpu.make_async_copy(xs.at[bg], xs.at[bg], xsem.at[bg]).wait()

    def o_copy(bg):
        b, g = bg // 4, bg % 4
        return pltpu.make_async_copy(
            os_.at[bg % 2], o_hbm.at[b, :, pl.ds(g * 128, 128)], osem.at[bg % 2])

    e_copy = pltpu.make_async_copy(we_hbm, wes, esem)

    def finalize(s1, s2, emb, gamma, beta, idx):
        inv = 1.0 / 4096.0
        m = jnp.sum(s1, axis=0, keepdims=True) * inv
        v = jnp.maximum(jnp.sum(s2, axis=0, keepdims=True) * inv - m * m, 0.0)
        if emb is not None:
            m = m + emb
        mu = jnp.sum(m, axis=1, keepdims=True) * (1.0 / 128.0)
        dm = m - mu
        var = jnp.sum(v + dm * dm, axis=1, keepdims=True) * (1.0 / 128.0)
        sc = lax.rsqrt(var + EPS) * gamma * 0.5
        sh = (0.5 * beta) - (mu if emb is None else mu - emb) * sc
        cf[idx, 0] = jnp.broadcast_to(sc, (8, 128))
        cf[idx, 1] = jnp.broadcast_to(sh, (8, 128))

    COST_X = 64 * 32 + 20

    def x_stats(bg):
        g = bg % 4
        s1 = s2 = None
        for r in range(64):
            w = xw[bg, pl.ds(r * 32, 32), :]
            lo, hi = _lo(w), _hi(w)
            a = _add(lo, hi)
            q = _add(lax.mul(lo, lo), lax.mul(hi, hi))
            a = _add(a[:16], a[16:])
            q = _add(q[:16], q[16:])
            a = _add(a[:8], a[8:])
            q = _add(q[:8], q[8:])
            s1 = a if s1 is None else _add(s1, a)
            s2 = q if s2 is None else _add(s2, q)
            yield 32, [s1, s2], True
        finalize(s1, s2, None, par[0, g], par[1, g], bg)
        yield 20, [], True

    def cost_a(src_x):
        return 64 * ((48 if src_x else 40) + 40) + 96 * 42

    def in_stage(src_x, bg, vb):
        g = bg % 4
        idx = bg if src_x else bg + 8
        sc, sh = cf[idx, 0], cf[idx, 1]
        sc, sh = _cat(sc, sc), _cat(sh, sh)
        sub = lax.broadcasted_iota(jnp.int32, (8, 128), 0)
        first, last = sub == 0, sub == 7
        zero = jnp.zeros((8, 128), F32)

        def row(h):
            if src_x:
                w = [xw[bg, pl.ds(h * 32 + k, 8, stride=4), :] for k in range(4)]
                w02, w13 = _cat(w[0], w[2]), _cat(w[1], w[3])
                y = [_lo(w02), _hi(w02), _lo(w13), _hi(w13)]
            else:
                y = [hs[bg, h, j] for j in range(4)]
            a = []
            for yj in y:
                u = _add(lax.mul(yj, sc), sh)
                a.append(_add(u, lax.mul(u, lax.tanh(u))))
            yield (48 if src_x else 40), [a[3][8:]], False
            left = lax.select(first, zero, pltpu.roll(a[3][8:], 1, 0))
            right = lax.select(last, zero, pltpu.roll(a[0][:8], 7, 0))
            r = _in_tf(_cat(left, a[3][:8]), a[0], a[1], a[2], a[3], _cat(a[0][8:], right))
            for jj in range(6):
                ts[h + 1, jj] = r[jj]
            yield 40, [r[4][8:]], True

        def col(th, jj):
            r = _in_tf(*[ts[4 * th + i, jj] for i in range(6)])
            for ii in range(6):
                vs[vb, ii * 6 + jj, g, pl.ds(th * 16, 16), :] = r[ii].astype(BF16)
            yield 42, [r[4][8:]], True

        h = 0
        for th in range(16):
            while h < min(64, 4 * th + 6):
                yield from row(h)
                h += 1
            for jj in range(6):
                yield from col(th, jj)

    COST_C1 = 32 * (96 + 4 * 28) + 20
    COST_C2 = 32 * (96 + 2 * (32 + 40))

    def out_rows(mb, th, e, z):
        rows = pl.ds(th * 16 + e * 8, 8)
        for i in range(6):
            z.append(_out_tf(*[ms[mb, i * 6 + j, rows, :] for j in range(6)]))
            yield 16, ([z[-1][3]] if i % 2 else []), False

    def out_stage1(mb, bg):
        b, g = bg // 4, bg % 4
        s1 = s2 = None
        for th in range(16):
            for e in range(2):
                z = []
                yield from out_rows(mb, th, e, z)
                for q in range(4):
                    y = _out_tf(*[z[i][q] for i in range(6)])
                    for p in range(4):
                        hs[bg, 4 * th + p, q, pl.ds(e * 8, 8), :] = y[p]
                    a = _add(_add(y[0], y[1]), _add(y[2], y[3]))
                    sq = [lax.mul(v, v) for v in y]
                    c = _add(_add(sq[0], sq[1]), _add(sq[2], sq[3]))
                    s1 = a if s1 is None else _add(s1, a)
                    s2 = c if s2 is None else _add(s2, c)
                    yield 28, ([s1, s2] if q == 3 else [s2]), q == 3
        finalize(s1, s2, par[4 + b, g], par[2, g], par[3, g], bg + 8)
        yield 20, [], True

    def out_stage2(mb, bg):
        for th in range(16):
            for e in range(2):
                z = []
                yield from out_rows(mb, th, e, z)
                for kq in range(2):
                    y0 = _out_tf(*[z[i][2 * kq] for i in range(6)])
                    y1 = _out_tf(*[z[i][2 * kq + 1] for i in range(6)])
                    yield 32, [y1[3]], False
                    for p in range(4):
                        rows = pl.ds((4 * th + p) * 32 + 2 * e + kq, 8, stride=4)
                        w = xw[bg, rows, :]
                        v = _cat(_add(y0[p], _lo(w)), _add(y1[p], _hi(w)))
                        v = lax.bitcast_convert_type(v.astype(BF16).astype(F32), U32)
                        v = lax.bitwise_or(
                            lax.shift_right_logical(v[:8], np.uint32(16)), v[8:])
                        ow[bg % 2, rows, :] = v
                    yield 40, [v], kq == 1

    COST_UK = 8 * (18 + 48 + 2 * 30 + 4 * 36)

    def w_stage(c, ks):
        for k in ks:
            for r in range(8):
                def emit(jj, t):
                    u = _w_tf(*t)
                    for ii in range(6):
                        us[c, ii * 6 + jj, k, pl.ds(r * 16, 16), :] = u[ii].astype(BF16)
                    return [u[4][8:]]
                g = [ws[c, k, t, pl.ds(r * 16, 16), :].astype(F32) for t in range(9)]
                yield 18 + 30, emit(0, g[0::3]), False
                yield 30, emit(5, g[2::3]), False
                eo = [_w_eo(g[3 * i], g[3 * i + 1], g[3 * i + 2]) for i in range(3)]
                yield 48, [eo[2][2][8:]], False
                yield 36, emit(1, [_add(v[0], v[1]) for v in eo]), False
                yield 36, emit(2, [_sub(v[0], v[1]) for v in eo]), False
                yield 36, emit(3, [_add(v[2], v[3]) for v in eo]), False
                yield 36, emit(4, [_sub(v[2], v[3]) for v in eo]), True

    NSUB = 16
    LEAD = 1

    def mm_stage(vb, c, mb, tasks):
        filler = _merge(tasks)
        total = sum(t[1] for t in tasks)
        keep = ts[0, 0, 0:8, :] == 0.0
        n = 128 // NSUB
        spent, nslot = 0, 36 * NSUB
        pend = []
        for ij in range(36):
            blocks = [[] for _ in range(4)]
            for r in range(NSUB):
                slot = ij * NSUB + r
                while spent < total * (slot + 1 - LEAD) / (nslot - LEAD):
                    cost, anchors, _ = next(filler)
                    spent += cost
                    pend.extend(anchors)
                for k in range(4):
                    w = vw[vb, ij, k, pl.ds(r * n, n), :]
                    if pend:
                        head = lax.select(
                            keep, w[:8], lax.bitcast_convert_type(pend.pop(0), U32))
                        w = _cat(head, w[8:]) if n > 8 else head
                    blocks[k].append(w)
            lhs = lax.concatenate(
                [pltpu.bitcast(lax.concatenate(b, 0), BF16) for b in blocks], 1)
            rhs = lax.concatenate([pltpu.bitcast(uw[c, ij, k], BF16) for k in range(4)], 1)
            ms[mb, ij] = lax.dot_general(lhs, rhs, (((1,), (1,)), ((), ())),
                                         preferred_element_type=F32)
        _run(filler)

    def step(s):
        u = s // 4
        tasks = []
        if s < 4:
            tasks.append((_chain(x_stats(s + 4), in_stage(True, s + 4, 1)),
                          COST_X + cost_a(True)))
        elif s < 12:
            tasks.append((in_stage(False, s - 4, (u + 1) % 2), cost_a(False)))
        if 1 <= s <= 8:
            tasks.append((out_stage1((s - 1) % 2, s - 1), COST_C1))
        elif s > 8:
            tasks.append((out_stage2((s - 1) % 2, s - 9), COST_C2))
        if s < 3:
            tasks.append((w_stage(s + 1, range(4)), 4 * COST_UK))
        elif s < 11:
            half = (s - 3) % 2
            tasks.append((w_stage(4 + (s - 3) // 2, (2 * half, 2 * half + 1)), 2 * COST_UK))
        mm_stage(u % 2, (u // 2) * 4 + s % 4, s % 2, tasks)

    for bg in range(4):
        x_copy(bg).start()
    w_start(0)
    for i, ref in enumerate((g1_ref, be1_ref, g2_ref, be2_ref)):
        v = ref[...].astype(F32)
        for g in range(4):
            par[i, g] = v[:, g * 128:(g + 1) * 128]
    ts[0] = jnp.zeros((6, 16, 128), F32)
    ts[65] = jnp.zeros((6, 16, 128), F32)

    def pro(g, carry):
        x_wait(g)

        @pl.when(g == 1)
        def _():
            x_copy(4).start()
            w_start(1)
            e_copy.start()

        _run(x_stats(g))
        _run(in_stage(True, g, 0))
        return carry + 1

    cnt = lax.fori_loop(0, 4, pro, 0)
    for bg in range(5, 8):
        x_copy(bg).start()
    for c in range(2, 8):
        w_start(c)
    w_wait(0)
    _run(w_stage(0, range(4)))
    e_copy.wait()
    t = t_ref[...].astype(F32)
    t = (t * jax.nn.sigmoid(t)).astype(BF16)
    emb = jnp.dot(t, wes[...], preferred_element_type=F32)
    for b in range(2):
        for g in range(4):
            par[4 + b, g] = emb[b:b + 1, g * 128:(g + 1) * 128]

    SPLIT = 1
    for s in range(16):
        if s < 4:
            x_wait(s + 4)
        if s <= 3:
            w_wait(s + 1)
        elif s in (5, 7, 9):
            w_wait(4 + (s - 3) // 2)
        if s >= 11:
            o_copy(s - 11).wait()
        if SPLIT:
            pl.when(cnt > s - 16)(lambda: step(s))
        else:
            step(s)
        if s >= 9:
            o_copy(s - 9).start()
    o_copy(5).wait()
    _run(out_stage2(1, 7))
    o_copy(7).start()
    o_copy(6).wait()
    o_copy(7).wait()


@jax.jit
def pallas_standalone__adm_resblock__diffusion_kernel(
        x, t_emb, g1, be1, w1, w_emb, g2, be2, w2):
    B, C, H, W = x.shape
    E = t_emb.shape[1]
    assert (B, C, H, W) == (2, 512, 64, 64)
    xt = x.transpose(0, 2, 3, 1).reshape(B, H * W, C)
    w1t = w1.transpose(2, 3, 0, 1).reshape(9, C, C)
    w2t = w2.transpose(2, 3, 0, 1).reshape(9, C, C)
    hbm = pl.BlockSpec(memory_space=pl.ANY)
    vm = pl.BlockSpec(memory_space=pltpu.VMEM)
    r = lambda a: a.reshape(1, C)
    out = pl.pallas_call(
        _kernel,
        out_shape=jax.ShapeDtypeStruct((B, H * W, C), x.dtype),
        in_specs=[hbm, vm, vm, vm, hbm, hbm, vm, vm, hbm],
        out_specs=hbm,
        scratch_shapes=[
            pltpu.VMEM((8, 4096, 128), BF16),
            pltpu.VMEM((8, 4, 9, 128, 128), BF16),
            pltpu.VMEM((E, C), BF16),
            pltpu.VMEM((8, 36, 4, 128, 128), BF16),
            pltpu.VMEM((2, 36, 4, 256, 128), BF16),
            pltpu.VMEM((2, 36, 256, 128), F32),
            pltpu.VMEM((8, 64, 4, 16, 128), F32),
            pltpu.VMEM((66, 6, 16, 128), F32),
            pltpu.VMEM((2, 4096, 128), BF16),
            pltpu.VMEM((6, 4, 1, 128), F32),
            pltpu.VMEM((16, 2, 8, 128), F32),
            pltpu.SemaphoreType.DMA((8,)),
            pltpu.SemaphoreType.DMA((8,)),
            pltpu.SemaphoreType.DMA(()),
            pltpu.SemaphoreType.DMA((2,)),
        ],
        compiler_params=pltpu.CompilerParams(vmem_limit_bytes=124 * 2 ** 20),
        name="resblock",
    )(xt, t_emb, r(g1), r(be1), w1t, w_emb, r(g2), r(be2), w2t)
    return out.reshape(B, H, W, C).transpose(0, 3, 1, 2)
```

```python
import jax
import jax.numpy as jnp
import numpy as np
from jax import lax
import jax.experimental.pallas as pl
import jax.experimental.pallas.tpu as pltpu

F32, BF16, U32 = jnp.float32, jnp.bfloat16, jnp.uint32

PA, PB = 1.5, 2.0 / 3.0
NA = 2.0 * PA * PA * (PA * PA - PB * PB)
NB = 2.0 * PB * PB * (PB * PB - PA * PA)
EPS = 1e-5

JJ_ORDER = (0, 5, 1, 2, 3, 4)
ALL = (0, 1, 2, 3)
JOBS = (
    (0, (0,), ALL, False), (0, (1,), ALL, True), (0, (2,), ALL, True), (0, (3,), ALL, True),
    (1, (0, 1), (0, 1), False), (1, (0, 1), (2, 3), False),
    (1, (2, 3), (0, 1), True), (1, (2, 3), (2, 3), True),
    (2, ALL, (0,), False), (2, ALL, (1,), False), (2, ALL, (2,), False), (2, ALL, (3,), False),
    (3, ALL, (0,), False), (3, ALL, (1,), False), (3, ALL, (2,), False), (3, ALL, (3,), False),
)
FENCES = (10, 30, 58, 89, 144, 180, 216, 288, 360, 432, 500, 556)
BY_COLUMN = (0,)
NMM = 36 * len(JOBS)
MARGIN = 2
LATENCY = 4
STREAM_RATE = 600
MAX_RATE = 52
MIN_RATE = 45


def u_slot(c, n):
    return n if c == 0 else (n + 4) % 5


def _mul(x, c):
    return lax.mul(x, np.float32(c))


_add, _sub = lax.add, lax.sub


def _in_tf(d0, d1, d2, d3, d4, d5):
    p = _mul(d2, PB * PB)
    q = _mul(d2, PA * PA)
    e1 = _sub(d4, p)
    e2 = _sub(d4, q)
    r0 = _add(_sub(d0, q), e1)
    t = _mul(d3, PB * PB)
    o1 = _sub(_mul(d3, PA * PA), d1)
    o2 = _sub(t, d1)
    r5 = _sub(_sub(d5, t), o1)
    o1 = _mul(o1, PB)
    o2 = _mul(o2, PA)
    return r0, _add(e1, o1), _sub(e1, o1), _add(e2, o2), _sub(e2, o2), r5


def _out_tf(m0, m1, m2, m3, m4, m5):
    s1, d1 = _add(m1, m2), _sub(m1, m2)
    s2, d2 = _add(m3, m4), _sub(m3, m4)
    y0 = _add(_add(m0, s1), s2)
    y1 = _add(_mul(d1, PA), _mul(d2, PB))
    y2 = _add(_mul(s1, PA * PA), _mul(s2, PB * PB))
    y3 = _add(_add(_mul(d1, PA ** 3), _mul(d2, PB ** 3)), m5)
    return y0, y1, y2, y3


def _w_eo(g0, g1, g2, p, n):
    return _add(_mul(g0, 1.0 / n), _mul(g2, p * p / n)), _mul(g1, p / n)


def _w_tf(g0, g1, g2):
    ea, oa = _w_eo(g0, g1, g2, PA, NA)
    eb, ob = _w_eo(g0, g1, g2, PB, NB)
    return g0, _add(ea, oa), _sub(ea, oa), _add(eb, ob), _sub(eb, ob), g2


def _lo(w):
    return lax.bitcast_convert_type(lax.shift_left(w, np.uint32(16)), F32)


def _hi(w):
    return lax.bitcast_convert_type(lax.bitwise_and(w, np.uint32(0xFFFF0000)), F32)


def _cat(a, b):
    return lax.concatenate([a, b], 0)


class _Piece:
    def __init__(self, emit, costs, deadline, release=-1, after=None):
        self.emit, self.costs = emit, costs
        self.deadline = deadline
        self.release = release
        self.after = after
        self.time = None


def _plan(streams):
    for st in streams:
        for p in st:
            p.soft = float(p.deadline)
    for _ in range(4):
        for st in streams:
            for i in reversed(range(len(st))):
                p = st[i]
                start = p.soft - sum(p.costs) / STREAM_RATE
                if i:
                    st[i - 1].deadline = min(st[i - 1].deadline, p.deadline)
                    st[i - 1].soft = min(st[i - 1].soft, start)
                if p.after is not None:
                    p.after.deadline = min(p.after.deadline, p.deadline)
                    p.after.soft = min(p.after.soft, start - LATENCY)
    due = np.zeros(NMM + 2)
    for st in streams:
        for p in st:
            p.bin = min(max(int(np.ceil(p.soft)), 1), max(p.deadline, 0))
            due[p.bin] += sum(p.costs)
    adds = np.array([2 * len(j[2]) * (len(j[1]) - (0 if j[3] else 1))
                     for j in JOBS for _ in range(36)])
    pos = [0] * len(streams)
    plan = [[] for _ in range(16 * NMM + 2)]
    cur, credit, rate = None, 0.0, 0.0

    def pick(mm):
        best = None
        for i, st in enumerate(streams):
            if pos[i] == len(st):
                continue
            p = st[pos[i]]
            urgent = p.deadline <= max(mm, 0) or mm > NMM
            if not urgent and (mm < 0 or p.release + MARGIN > mm):
                continue
            if p.after is not None and (p.after.time is None or (
                    not urgent and p.after.time + LATENCY > mm)):
                continue
            key = (not urgent, p.soft)
            if best is None or key < best[0]:
                best = key, i
        return best

    for slot in range(-1, 16 * NMM + 1):
        mm = slot // 16 if slot < 16 * NMM else NMM + 1
        if 0 <= mm < NMM:
            if slot % 16 == 0:
                due[mm + 1] += due[1:mm + 1].sum()
                due[1:mm + 1] = 0
                need = np.cumsum(due[mm + 1:NMM + 1] + 16 * adds[mm:])
                rate = np.max(need / (16.0 * np.arange(1, NMM - mm + 1)))
                rate = min(max(rate, MIN_RATE), MAX_RATE) - adds[mm]
            credit += rate
        left = min([16 * f - 1 - slot for f in FENCES if 16 * f > slot], default=1000)
        while True:
            if cur is None:
                best = pick(mm)
                if best is None:
                    credit = min(credit, 0.0)
                    break
                i = best[1]
                p = streams[i][pos[i]]
                if best[0][0] and (credit <= 0 or sum(p.costs) > credit + left * rate):
                    break
                assert p.release < max(mm, 0), (i, pos[i], p.release, mm)
                pos[i] += 1
                cur = [p, 0]
            p, k = cur
            best = pick(mm)
            if credit <= 0 and left and p.deadline > max(mm, 0) and mm <= NMM and (
                    best is None or best[0][0]):
                break
            plan[slot + 1].append(p)
            credit = max(credit - p.costs[k], -64.0) if mm >= 0 else 0.0
            due[max(p.bin, min(mm + 1, NMM + 1)) if p.bin else 0] -= p.costs[k]
            cur[1] += 1
            if cur[1] == len(p.costs):
                p.time, cur = mm, None
    assert all(n == len(st) for n, st in zip(pos, streams))
    return plan


def _kernel(x_hbm, t_hbm, g1_hbm, be1_hbm, w1_hbm, we_hbm, g2_hbm, be2_hbm, w2_hbm,
            o_hbm,
            xs, ws, wes, tv, gv, us, v0, v1, ms, hs, ts, emb_s, acc_s, cf,
            xsem, wsem, psem, osem):
    xw = xs.bitcast(U32)
    uw = us.bitcast(U32)
    vs = (v0, v1)
    vw = (v0.bitcast(U32), v1.bitcast(U32))

    def x_copy(bg, part=None):
        rows = slice(None) if part is None else pl.ds(1024 * part, 1024)
        return pltpu.make_async_copy(
            x_hbm.at[bg // 4, rows, pl.ds(bg % 4 * 128, 128)], xs.at[bg, rows],
            xsem.at[bg if part is None else 8 + part])

    def w_copy(c, k):
        return pltpu.make_async_copy(
            (w1_hbm, w2_hbm)[c].at[:, :, :, pl.ds(k * 128, 128)], ws.at[c, k],
            wsem.at[4 * c + k])

    def o_copy(bg, part=None):
        rows = slice(None) if part is None else pl.ds(1024 * part, 1024)
        return pltpu.make_async_copy(
            xs.at[bg, rows], o_hbm.at[bg // 4, rows, pl.ds(bg % 4 * 128, 128)],
            osem.at[bg if part is None else 8 + part])

    p_copy = [pltpu.make_async_copy(src, dst, psem.at[i]) for i, (src, dst) in enumerate(
        ((g1_hbm, gv[0]), (be1_hbm, gv[1]), (g2_hbm, gv[2]), (be2_hbm, gv[3]),
         (t_hbm, tv), (we_hbm, wes)))]

    def start_rest():
        for cp in fences[10]:
            cp.start()
        yield []

    def waiting(*copies):
        def emit():
            for cp in copies:
                cp.wait()
            yield []
        return _Piece(emit, [1], NMM + 1)

    def uses(pred):
        t = [36 * s + 6 * n + ii for s, job in enumerate(JOBS)
             for n, jj in enumerate(JJ_ORDER) for ii in range(6) if pred(job, jj)]
        return min(t), max(t)

    latest = []

    def finalize(idx):
        def emit():
            coefficients(idx)
            yield []
        return _Piece(emit, [30], NMM + 1)

    def coefficients(idx):
        g = idx % 4
        s1, s2 = acc_s[idx, 0], acc_s[idx, 1]
        if latest:
            s1 = lax.select(ts[0, 0, 0:8, :] > 1.0, latest[-1], s1)
        emb = emb_s[pl.ds(idx // 4 - 2, 1), pl.ds(128 * g, 128)] if idx >= 8 else None
        gamma, beta = (r[...].astype(F32).reshape(1, 512)[:, 128 * g:128 * (g + 1)]
                       for r in gv[idx // 8 * 2:idx // 8 * 2 + 2])
        inv = 1.0 / 4096.0
        m = jnp.sum(s1, axis=0, keepdims=True) * inv
        v = jnp.maximum(jnp.sum(s2, axis=0, keepdims=True) * inv - m * m, 0.0)
        if emb is not None:
            m = m + emb
        mu = jnp.sum(m, axis=1, keepdims=True) * (1.0 / 128.0)
        dm = m - mu
        var = jnp.sum(v + dm * dm, axis=1, keepdims=True) * (1.0 / 128.0)
        sc = lax.rsqrt(var + EPS) * gamma * 0.5
        sh = (0.5 * beta) - (mu if emb is None else mu - emb) * sc
        cf[idx, 0] = jnp.broadcast_to(sc, (8, 128))
        cf[idx, 1] = jnp.broadcast_to(sh, (8, 128))

    def x_stats(bg):
        def part(n):
            def emit():
                acc = [acc_s[bg, 0], acc_s[bg, 1]] if n else [None, None]
                if latest:
                    xw[8, 0:8, :] = lax.bitcast_convert_type(latest[-1], U32)
                for r in range(8 * n, 8 * n + 8):
                    w = xw[bg + zero if latest else bg, pl.ds(r * 32, 32), :]
                    lo, hi = _lo(w), _hi(w)
                    a = _add(lo, hi)
                    q = _add(lax.mul(lo, lo), lax.mul(hi, hi))
                    for i, v in enumerate((a, q)):
                        v = _add(v[:16], v[16:])
                        v = _add(v[:8], v[8:])
                        acc[i] = v if acc[i] is None else _add(acc[i], v)
                    if r % 8 == 7:
                        acc[0] = lax.select(ts[0, 0, 0:8, :] == 0.0, acc[0], acc[1])
                        acc_s[bg, 0], acc_s[bg, 1] = acc
                    yield list(acc)
            return _Piece(emit, [32] * 8, NMM + 1)

        out = []
        for n in range(8):
            if bg == 0 and n % 2 == 0:
                out.append(waiting(x_copy(0, n // 2)))
            out.append(part(n))
        if bg == 0:
            out += [waiting(*p_copy[:2]), _Piece(start_rest, [1], NMM + 1)]
        return out + [finalize(bg)]

    def in_stage(idx, stats):
        unit, g = idx // 4, idx % 4

        def row(h):
            def emit():
                sc, sh = cf[idx, 0], cf[idx, 1]
                sc, sh = _cat(sc, sc), _cat(sh, sh)
                if idx < 8:
                    w = [xw[idx, pl.ds(h * 32 + k, 8, stride=4), :] for k in range(4)]
                    w02, w13 = _cat(w[0], w[2]), _cat(w[1], w[3])
                    y = [_lo(w02), _hi(w02), _lo(w13), _hi(w13)]
                else:
                    y = [hs[idx - 8, h, j] for j in range(4)]
                a = []
                for yj in y:
                    u = _add(lax.mul(yj, sc), sh)
                    a.append(_add(u, lax.mul(u, lax.tanh(u))))
                yield [a[3][8:]]
                sub = lax.broadcasted_iota(jnp.int32, (8, 128), 0)
                pad = jnp.zeros((8, 128), F32)
                left = lax.select(sub == 0, pad, pltpu.roll(a[3][8:], 1, 0))
                right = lax.select(sub == 7, pad, pltpu.roll(a[0][:8], 7, 0))
                r = _in_tf(_cat(left, a[3][:8]), a[0], a[1], a[2], a[3], _cat(a[0][8:], right))
                for jj in range(6):
                    ts[h + 1, jj] = r[jj]
                yield [r[4][:8], r[4][8:]]
            return _Piece(emit, [48 if idx < 8 else 40, 40], NMM + 1, after=stats)

        def col(th, jj, deadline, release):
            def emit():
                r = _in_tf(*[ts[4 * th + i, jj] for i in range(6)])
                for ii in range(6):
                    vs[unit % 2][ii * 6 + jj, g, pl.ds(th * 16, 16), :] = r[ii].astype(BF16)
                yield [r[4][:8], r[4][8:]]
            return _Piece(emit, [42], deadline, release)

        when = {}
        for jj in JJ_ORDER:
            first = uses(lambda j, q: j[0] == unit and g in j[1] and q == jj)[0]
            prev = -1 if unit < 2 else uses(
                lambda j, q: j[0] == unit - 2 and g in j[1] and q == jj)[1]
            when[jj] = first - MARGIN, prev
        if idx in BY_COLUMN:
            return [row(h) for h in range(64)] + [
                col(th, jj, *when[jj]) for jj in JJ_ORDER for th in range(16)]
        out = [row(h) for h in range(6)]
        if unit >= 2:
            out[0].release = {2: 216, 3: 360}[unit] - MARGIN
        for th in range(16):
            out += [col(th, jj, *when[jj]) for jj in JJ_ORDER]
            out += [row(h) for h in range(4 * th + 6, min(64, 4 * th + 10))]
        return out

    def out_stage(idx):
        unit, g = idx // 4, idx % 4
        bg = idx % 8
        last = uses(lambda j, q: j[0] == unit and g in j[2])[1]
        mb = idx % 8
        deadline = (216, 360)[unit] if unit < 2 else out_block[bg]

        def rows(th, e, z):
            r = pl.ds(th * 16 + e * 8, 8)
            for i in range(6):
                z.append(_out_tf(*[ms[mb, i * 6 + j, r, :] for j in range(6)]))
                yield [z[-1][3]]

        def hidden(th, e):
            def emit():
                z = []
                yield from rows(th, e, z)
                acc = [acc_s[idx + 8, 0], acc_s[idx + 8, 1]] if th or e else [None, None]
                for q in range(4):
                    y = _out_tf(*[z[i][q] for i in range(6)])
                    for p in range(4):
                        hs[bg, 4 * th + p, q, pl.ds(e * 8, 8), :] = y[p]
                    sq = [lax.mul(v, v) for v in y]
                    for i, v in enumerate((y, sq)):
                        v = _add(_add(v[0], v[1]), _add(v[2], v[3]))
                        acc[i] = v if acc[i] is None else _add(acc[i], v)
                    if q == 3:
                        acc[0] = lax.select(ts[0, 0, 0:8, :] == 0.0, acc[0], acc[1])
                        acc_s[idx + 8, 0], acc_s[idx + 8, 1] = acc
                    yield acc[:1] if q == 3 else acc[1:]
            return _Piece(emit, [16] * 6 + [28] * 4, deadline, last)

        def final(th, e):
            def emit():
                z = []
                yield from rows(th, e, z)
                for kq in range(2):
                    y0 = _out_tf(*[z[i][2 * kq] for i in range(6)])
                    y1 = _out_tf(*[z[i][2 * kq + 1] for i in range(6)])
                    yield [y1[3]]
                    for p in range(4):
                        r = pl.ds((4 * th + p) * 32 + 2 * e + kq, 8, stride=4)
                        w = xw[bg, r, :]
                        v = _cat(_add(y0[p], _lo(w)), _add(y1[p], _hi(w)))
                        v = lax.bitcast_convert_type(v.astype(BF16).astype(F32), U32)
                        v = lax.bitwise_or(
                            lax.shift_right_logical(v[:8], np.uint32(16)), v[8:])
                        xw[bg, r, :] = v
                    if bg == 7 and th % 4 == 3 and e == 1 and kq == 1:
                        o_copy(7, th // 4).start()
                    yield [v]
            return _Piece(emit, [16] * 6 + [32, 40] * 2, deadline, last)

        if unit < 2:
            fin = finalize(idx + 8)
            fin.after = emb_stream[-1]
            fin.deadline = (216, 360)[unit]
            return [hidden(th, e) for th in range(16) for e in range(2)] + [fin]
        return [final(th, e) for th in range(16) for e in range(2)]

    def w_stage(c, n, k, phases):
        def piece(r, jjs):
            def emit():
                def out(jj, t):
                    u = _w_tf(*t)
                    for ii in range(6):
                        us[u_slot(c, n), ii * 6 + jj, k, pl.ds(r * 16, 16), :] = u[ii].astype(BF16)
                    return [u[i][h:h + 8] for i in ((2, 4) if jj in (0, 5) else (4,))
                            for h in (0, 8)]

                def tap(j):
                    return [ws[c, k if jjs[0] in (0, 5) else k + zero * jjs[0],
                               i, j, pl.ds(128 * n + 16 * r, 16), :].astype(F32)
                            for i in range(3)]
                if jjs != (5,):
                    g0 = tap(0)
                if 0 in jjs:
                    yield out(0, g0)
                if jjs != (0,):
                    g2 = tap(2)
                if 5 in jjs:
                    yield out(5, g2)
                if 1 in jjs or 3 in jjs:
                    g1 = tap(1)
                    eo = {jj: [_w_eo(*v, p, nrm) for v in zip(g0, g1, g2)]
                          for jj, p, nrm in ((1, PA, NA), (3, PB, NB)) if jj in jjs}
                    for jj in reversed(eo):
                        yield out(jj, [_add(*v) for v in eo[jj]])
                        yield out(jj + 1, [_sub(*v) for v in eo[jj]])
            return emit

        res = []
        for jjs in phases:
            first = uses(lambda j, q: j[0] // 2 == c and k in j[1] and n in j[2] and q in jjs)[0]
            prev = -1 if c == 0 or n == 0 else 288 - MARGIN
            prev = max(prev, w_ready[4 * c + k])
            costs = {1: [36], 2: [78, 36], 6: [36, 36, 90, 36, 36, 36]}[len(jjs)]
            res += [_Piece(piece(r, jjs), costs, first - MARGIN - 1, prev) for r in range(8)]
        return res

    def emb_part(e, release):
        def emit():
            t = tv[:, pl.ds(128 * e, 128)].astype(F32)
            t = (t * jax.nn.sigmoid(t)).astype(BF16)
            v = jnp.dot(t, wes[pl.ds(128 * e, 128), :], preferred_element_type=F32)
            emb_s[...] = emb_s[...] + v if e else v
            yield []
        return _Piece(emit, [20], release + 2, release)

    fences = {
        10: [x_copy(1)],
        30: [w_copy(0, 1), x_copy(2)],
        58: [w_copy(0, 2), x_copy(3)],
        89: [w_copy(0, 3), x_copy(4), x_copy(5)],
        144: [x_copy(6), x_copy(7), *p_copy[2:]],
        216: [w_copy(1, k) for k in ALL],
    }
    starts = {10: fences[30], 30: fences[58], 58: fences[89],
              89: [x_copy(6), x_copy(7), p_copy[5]], 144: fences[216]}
    x_ready = [f - MARGIN for f in (1, 10, 30, 58, 89, 89, 144, 144)]
    w_ready = [f - MARGIN for f in (1, 30, 58, 89, 216, 216, 216, 216)]
    out_block = (500, 500, 500, 500, 500, 556, 556, NMM + 1)
    emb_stream = [emb_part(e, 146 + 2 * e) for e in range(9)]
    stat_streams = [x_stats(bg) for bg in range(8)] + [out_stage(i) for i in range(8)]
    for bg in range(8):
        stat_streams[bg][0].release = x_ready[bg]
    in_stream = []
    for idx in range(16):
        in_stream += in_stage(idx, stat_streams[idx][-1])
        if idx == 0:
            for p in in_stream[:100]:
                p.deadline = 0
            in_stream.insert(100, waiting(w_copy(0, 0)))
            w_landed = in_stream[100]
    split, whole = ((0,), (5,), (1, 2), (3, 4)), (JJ_ORDER,)
    w_stream = []
    for k in ALL:
        for jjs in split:
            for n in ALL:
                w_stream += w_stage(0, n, k, (jjs,))
    w_stream[0].after = w_landed
    for n in ALL:
        for k in ALL:
            w_stream += w_stage(1, n, k, whole)
    plan = _plan(stat_streams + [in_stream, w_stream, emb_stream]
                 + [out_stage(i) for i in range(8, 16)])

    running = {}

    def advance(slot):
        pend = []
        for p in plan[slot + 1]:
            if id(p) not in running:
                running[id(p)] = p.emit()
            pend += next(running[id(p)])
        return pend

    def matmuls(lo, hi, zero):
        keeps = [ts[0, i, 0:8, :] == 0.0 for i in range(4)]
        for mm in range(lo, hi):
            s, t = divmod(mm, 36)
            unit, ks, ns, acc = JOBS[s]
            ij = (t % 6) * 6 + JJ_ORDER[t // 6]
            blocks = [[] for _ in ks]
            src = ij if s < 6 or 36 * s <= lo else ij + zero * (s % 4)
            whole = [vw[unit % 2][src, k] for k in ks]
            for r in range(16):
                pend = advance(16 * mm + r)
                w = [lax.slice(v, (8 * r, 0), (8 * r + 8, 128)) for v in whole]
                for i, a in enumerate(pend[-4 * len(ks):]):
                    w[i % len(ks)] = lax.select(
                        keeps[i // len(ks)], w[i % len(ks)], lax.bitcast_convert_type(a, U32))
                for b, v in zip(blocks, w):
                    b.append(v)
            lhs = lax.concatenate(
                [pltpu.bitcast(lax.concatenate(b, 0), BF16) for b in blocks], 1)
            rhs = lax.concatenate([lax.concatenate(
                [pltpu.bitcast(uw[u_slot(unit // 2, n), ij, k], BF16) for k in ks], 1) for n in ns], 0)
            res = lax.dot_general(lhs, rhs, (((1,), (1,)), ((), ())),
                                  preferred_element_type=F32)
            for i, n in enumerate(ns):
                mb = unit % 2 * 4 + n
                v = res[:, 128 * i:128 * (i + 1)]
                ms[mb, ij] = _add(ms[mb, ij], v) if acc else v
            latest[:] = [v[:8]] if mm + 1 < hi else []

    for cp in p_copy[:5]:
        cp.start()
    for n in range(4):
        x_copy(0, n).start()
    w_copy(0, 0).start()
    ts[0] = jnp.zeros((6, 16, 128), F32)
    ts[65] = jnp.zeros((6, 16, 128), F32)
    zero = lax.fori_loop(0, 3, lambda i, c: c + i, 0) - 3

    advance(-1)
    for lo, hi in zip((0,) + FENCES, FENCES + (NMM,)):
        for cp in fences.get(lo, ()):
            cp.wait()
        for cp in starts.get(lo, ()):
            cp.start()
        for bg in range(7):
            if out_block[bg] == lo:
                o_copy(bg).start()
        pl.when(zero <= lo)(lambda: matmuls(lo, hi, zero))
    advance(16 * NMM)
    for bg in range(7):
        o_copy(bg).wait()
    for n in range(4):
        o_copy(7, n).wait()


@jax.jit
def pallas_standalone__adm_resblock__diffusion_kernel(
        x, t_emb, g1, be1, w1, w_emb, g2, be2, w2):
    B, C, H, W = x.shape
    E = t_emb.shape[1]
    assert (B, C, H, W, E) == (2, 512, 64, 64, 1152)
    xt = x.transpose(0, 2, 3, 1).reshape(B, H * W, C)
    hbm = pl.BlockSpec(memory_space=pl.ANY)
    out = pl.pallas_call(
        _kernel,
        out_shape=jax.ShapeDtypeStruct((B, H * W, C), x.dtype),
        in_specs=[hbm] * 9,
        out_specs=hbm,
        scratch_shapes=[
            pltpu.VMEM((9, 4096, 128), BF16),
            pltpu.VMEM((2, 4, 3, 3, 512, 128), BF16),
            pltpu.VMEM((E, C), BF16),
            pltpu.VMEM((B, E), BF16),
            [pltpu.VMEM((C,), BF16)] * 4,
            pltpu.VMEM((5, 36, 4, 128, 128), BF16),
            pltpu.VMEM((36, 4, 256, 128), BF16),
            pltpu.VMEM((36, 4, 256, 128), BF16),
            pltpu.VMEM((8, 36, 256, 128), F32),
            pltpu.VMEM((8, 64, 4, 16, 128), F32),
            pltpu.VMEM((66, 6, 16, 128), F32),
            pltpu.VMEM((B, C), F32),
            pltpu.VMEM((16, 2, 8, 128), F32),
            pltpu.VMEM((16, 2, 8, 128), F32),
            pltpu.SemaphoreType.DMA((12,)),
            pltpu.SemaphoreType.DMA((8,)),
            pltpu.SemaphoreType.DMA((6,)),
            pltpu.SemaphoreType.DMA((12,)),
        ],
        compiler_params=pltpu.CompilerParams(vmem_limit_bytes=124 * 2 ** 20),
        name="resblock",
    )(xt, t_emb, g1, be1, w1.transpose(2, 3, 0, 1), w_emb, g2, be2, w2.transpose(2, 3, 0, 1))
    return out.reshape(B, H, W, C).transpose(0, 3, 1, 2)
```

```python
import jax
import jax.numpy as jnp
import numpy as np
from jax import lax
import jax.experimental.pallas as pl
import jax.experimental.pallas.tpu as pltpu

F32, BF16, U32 = jnp.float32, jnp.bfloat16, jnp.uint32

PA, PB = 1.5, 2.0 / 3.0
NA = 2.0 * PA * PA * (PA * PA - PB * PB)
EPS = 1e-5

JJ_ORDER = (0, 5, 1, 2, 3, 4)
ALL = (0, 1, 2, 3)
JOBS = (
    (0, (0,), ALL, False), (0, (1,), ALL, True), (0, (2,), ALL, True), (0, (3,), ALL, True),
    (1, (0, 1), (0, 1), False), (1, (0, 1), (2, 3), False),
    (1, (2, 3), (0, 1), True), (1, (2, 3), (2, 3), True),
    (2, ALL, (0,), False), (2, ALL, (1,), False), (2, ALL, (2,), False), (2, ALL, (3,), False),
    (3, ALL, (0,), False), (3, ALL, (1,), False), (3, ALL, (2,), False), (3, ALL, (3,), False),
)
FENCES = (10, 24, 46, 89, 144, 180, 216, 288, 360, 432, 503, 555, 571, 574)
BY_COLUMN = (0, 4, 5, 7)
NMM = 36 * len(JOBS)
MARGIN = 2
LATENCY = 4
STREAM_RATE = 600
STORE_RATE = 139
ALU0 = 48
ALU1 = 46
ALU2 = 43
ALU3 = 40
ALU_RATE = (ALU0,) * 4 + (ALU1,) * 4 + (ALU2,) * 4 + (ALU3,) * 4


def u_slot(c, n):
    return n if c == 0 else (n + 4) % 5


_add, _sub = lax.add, lax.sub


def _mul(x, c):
    return x if abs(c - 1.0) < 1e-12 else lax.mul(x, np.float32(c))


IN_SCALE = (PA, PA * PA, PB, 1.0)
W_SCALE = PA ** 3 / NA ** 2


def _in_tf(d0, d1, d2, d3, d4, d5):
    p = _mul(d2, PB ** 4)
    ea, eb = _sub(d4, p), _sub(d4, d2)
    r0 = _add(_sub(d0, p), eb)
    t = _mul(d3, PA ** 4)
    oa, ob = _mul(_sub(t, d1), PB * PB), _sub(d3, d1)
    r5 = _sub(_sub(d5, t), ob)
    return r0, _add(ea, oa), _sub(ea, oa), _add(eb, ob), _sub(eb, ob), r5


def _out_tf(m0, m1, m2, m3, m4, m5):
    sa, da = _add(m1, m2), _sub(m1, m2)
    sb, db = _add(m3, m4), _sub(m3, m4)
    y0 = _sub(_add(m0, sa), _mul(sb, PA ** 4))
    y1 = _sub(da, _mul(db, PA * PA))
    y2 = _sub(sa, sb)
    y3 = _add(_sub(da, _mul(db, PB * PB)), m5)
    return y0, y1, y2, y3


def _w_tf(g0, g1, g2):
    ea = _add(g0, g2)
    eb, ob = _add(g0, _mul(g2, PB ** 4)), _mul(g1, PB * PB)
    return (_mul(g0, NA), _add(ea, g1), _sub(ea, g1), _add(eb, ob), _sub(eb, ob),
            _mul(g2, NA / PA ** 6))


def _lo(w):
    return lax.bitcast_convert_type(lax.shift_left(w, np.uint32(16)), F32)


def _hi(w):
    return lax.bitcast_convert_type(lax.bitwise_and(w, np.uint32(0xFFFF0000)), F32)


def _cat(a, b):
    return lax.concatenate([a, b], 0)


class _Piece:
    def __init__(self, emit, costs, deadline, release=-1, after=None):
        self.emit, self.costs = emit, np.array(costs, float)
        self.deadline = deadline
        self.release = release
        self.after = after
        self.time = None


def _plan(streams):
    for st in streams:
        for p in st:
            p.soft = float(p.deadline)
    for _ in range(4):
        for st in streams:
            for i in reversed(range(len(st))):
                p = st[i]
                start = p.soft - p.costs[:, 0].sum() / STREAM_RATE
                if i:
                    st[i - 1].deadline = min(st[i - 1].deadline, p.deadline)
                    st[i - 1].soft = min(st[i - 1].soft, start)
                if p.after is not None:
                    p.after.deadline = min(p.after.deadline, p.deadline)
                    p.after.soft = min(p.after.soft, start - LATENCY)
    pos = [0] * len(streams)
    plan = [[] for _ in range(16 * NMM + 2)]
    cur, credit, rate = None, np.zeros(2), np.zeros(2)

    def pick(mm):
        best = None
        for i, st in enumerate(streams):
            if pos[i] == len(st):
                continue
            p = st[pos[i]]
            urgent = p.deadline <= max(mm, 0) + (left == 0) or mm > NMM
            if not urgent and (mm < 0 or p.release + MARGIN > mm):
                continue
            if p.after is not None and (p.after.time is None or (
                    not urgent and p.after.time + LATENCY > mm)):
                continue
            key = (not urgent, credit[1] <= 0 and p.costs[:, 1].any(), p.soft)
            if best is None or key < best[0]:
                best = key, i
        return best

    def affordable(cost):
        return all(c > 0 or not need for c, need in zip(credit, cost))

    for slot in range(-1, 16 * NMM + 1):
        mm = slot // 16 if slot < 16 * NMM else NMM + 1
        if 0 <= mm < NMM:
            _, ks, ns, acc = JOBS[mm // 36]
            rate = np.array([ALU_RATE[mm // 36] - 2 * len(ns) * (len(ks) - (not acc)),
                             STORE_RATE / 10 - 2 * len(ns)])
            credit = np.minimum(credit + rate, 2 * rate)
        left = min([16 * f - 1 - slot for f in FENCES if 16 * f > slot], default=1000)
        while True:
            best = pick(mm)
            if cur is None:
                if best is None:
                    break
                i = best[1]
                p = streams[i][pos[i]]
                if best[0][0] and not (affordable(p.costs.sum(0)) and all(
                        p.costs.sum(0) <= credit + left * rate)):
                    break
                assert p.release < max(mm, 0) and (mm < p.deadline or mm not in FENCES)
                pos[i] += 1
                cur = [p, 0]
            p, k = cur
            if not affordable(p.costs[k]) and left and p.deadline > max(mm, 0) and (
                    mm <= NMM and (best is None or best[0][0])):
                break
            plan[slot + 1].append(p)
            credit = np.maximum(credit - p.costs[k], -2 * rate)
            cur[1] += 1
            if cur[1] == len(p.costs):
                p.time, cur = mm, None
    assert all(n == len(st) for n, st in zip(pos, streams))
    return plan


def _kernel(x_hbm, t_hbm, g1_hbm, be1_hbm, w1_hbm, we_hbm, g2_hbm, be2_hbm, w2_hbm,
            o_hbm,
            xs, os_, ws, wes, tv, gv, us, v0, v1, ms, hs, ts, emb_s, acc_s, cf,
            xsem, wsem, psem, osem):
    xw = xs.bitcast(U32)
    ow = os_.bitcast(U32)
    uw = us.bitcast(U32)
    vs = (v0, v1)
    vw = (v0.bitcast(U32), v1.bitcast(U32))

    def x_copy(bg, part=None):
        rows = slice(None) if part is None else pl.ds(4 * part, 4)
        return pltpu.make_async_copy(
            x_hbm.at[bg // 4, rows, :, :, pl.ds(bg % 4 * 128, 128)], xs.at[bg, rows],
            xsem.at[bg if part is None else 8 + part])

    def w_copy(c, k):
        return pltpu.make_async_copy(
            (w1_hbm, w2_hbm)[c].at[:, :, :, pl.ds(k * 128, 128)], ws.at[c, k],
            wsem.at[4 * c + k])

    def o_copy(bg, part=None):
        rows = slice(None) if part is None else pl.ds(part, 1)
        return pltpu.make_async_copy(
            os_.at[bg, :, rows], o_hbm.at[bg // 4, :, rows, :, pl.ds(bg % 4 * 128, 128)],
            osem.at[bg if part is None else 8 + part])

    p_copy = [pltpu.make_async_copy(src, dst, psem.at[i]) for i, (src, dst) in enumerate(
        ((g1_hbm, gv[0]), (be1_hbm, gv[1]), (g2_hbm, gv[2]), (be2_hbm, gv[3]),
         (t_hbm, tv), (we_hbm, wes)))]

    def start_rest():
        for cp in fences[10]:
            cp.start()
        yield []

    def waiting(*copies):
        def emit():
            for cp in copies:
                cp.wait()
            yield []
        return _Piece(emit, [(1, 0)], NMM + 1)

    def uses(pred):
        t = [36 * s + 6 * n + ii for s, job in enumerate(JOBS)
             for n, jj in enumerate(JJ_ORDER) for ii in range(6) if pred(job, jj)]
        return min(t), max(t)

    latest = []

    def finalize(idx):
        def emit():
            coefficients(idx)
            yield []
        return _Piece(emit, [(30, 0)], NMM + 1)

    def coefficients(idx):
        g = idx % 4
        s1, s2 = acc_s[idx, 0], acc_s[idx, 1]
        if latest:
            s1 = lax.select(ts[0, 0, 0:8, :] > 1.0, latest[-1], s1)
        emb = emb_s[pl.ds(idx // 4 - 2, 1), pl.ds(128 * g, 128)] if idx >= 8 else None
        gamma, beta = (r[...].astype(F32).reshape(1, 512)[:, 128 * g:128 * (g + 1)]
                       for r in gv[idx // 8 * 2:idx // 8 * 2 + 2])
        inv = 1.0 / 4096.0
        m = jnp.sum(s1, axis=0, keepdims=True) * inv
        v = jnp.maximum(jnp.sum(s2, axis=0, keepdims=True) * inv - m * m, 0.0)
        if emb is not None:
            m = m + emb
        mu = jnp.sum(m, axis=1, keepdims=True) * (1.0 / 128.0)
        dm = m - mu
        var = jnp.sum(v + dm * dm, axis=1, keepdims=True) * (1.0 / 128.0)
        sc = lax.rsqrt(var + EPS) * gamma * 0.5
        sh = (0.5 * beta) - (mu if emb is None else mu - emb) * sc
        cf[idx, 0] = jnp.broadcast_to(sc, (8, 128))
        cf[idx, 1] = jnp.broadcast_to(sh, (8, 128))

    def x_stats(bg):
        def part(n):
            def emit():
                acc = [acc_s[bg, 0], acc_s[bg, 1]] if n else [None, None]
                if latest:
                    xw[8, 0, 0, 0:8, :] = lax.bitcast_convert_type(latest[-1], U32)
                for r in range(8 * n, 8 * n + 8):
                    w = xw[bg + zero if latest else bg, r // 4, r % 4]
                    lo, hi = _lo(w), _hi(w)
                    a = _add(lo, hi)
                    q = _add(lax.mul(lo, lo), lax.mul(hi, hi))
                    for i, v in enumerate((a, q)):
                        v = _add(v[:16], v[16:])
                        v = _add(v[:8], v[8:])
                        acc[i] = v if acc[i] is None else _add(acc[i], v)
                    if r % 8 == 7:
                        acc[0] = lax.select(ts[0, 0, 0:8, :] == 0.0, acc[0], acc[1])
                        acc_s[bg, 0], acc_s[bg, 1] = acc
                    yield list(acc)
            return _Piece(emit, [(34, 0)] * 8, NMM + 1)

        out = []
        for n in range(8):
            if bg == 0 and n % 2 == 0:
                out.append(waiting(x_copy(0, n // 2)))
            out.append(part(n))
        if bg == 0:
            out += [waiting(*p_copy[:2]), _Piece(start_rest, [(1, 0)], NMM + 1)]
        return out + [finalize(bg)]

    def in_stage(idx, stats):
        unit, g = idx // 4, idx % 4

        def row(h):
            def emit():
                sc, sh = cf[idx, 0], cf[idx, 1]
                sc, sh = _cat(sc, sc), _cat(sh, sh)
                if idx < 8:
                    w = [xw[idx, h // 4, h % 4, pl.ds(k, 8, stride=4), :] for k in range(4)]
                    w02, w13 = _cat(w[0], w[2]), _cat(w[1], w[3])
                    y = [_lo(w02), _hi(w02), _lo(w13), _hi(w13)]
                else:
                    y = [hs[idx - 8, h, j] for j in range(4)]
                a = []
                for j, yj in enumerate(y):
                    u = _add(lax.mul(yj, sc), sh)
                    v = _mul(u, IN_SCALE[h % 4] * IN_SCALE[j])
                    a.append(_add(v, lax.mul(v, lax.tanh(u))))
                yield [a[3][8:]]
                sub = lax.broadcasted_iota(jnp.int32, (8, 128), 0)
                pad = jnp.zeros((8, 128), F32)
                left = lax.select(sub == 0, pad, pltpu.roll(a[3][8:], 1, 0))
                right = lax.select(sub == 7, pad, pltpu.roll(a[0][:8], 7, 0))
                r = _in_tf(_cat(left, a[3][:8]), a[0], a[1], a[2], a[3], _cat(a[0][8:], right))
                for jj in range(6):
                    ts[h + 1, jj] = r[jj]
                yield [r[4][:8], r[4][8:]]
            return _Piece(emit, [(47 if idx < 8 else 39, 0), (36, 12)], NMM + 1, after=stats)

        def col(th, jj, deadline, release):
            def emit():
                r = _in_tf(*[ts[4 * th + i, jj] for i in range(6)])
                for ii in range(6):
                    vs[unit % 2][ii * 6 + jj, g, pl.ds(th * 16, 16), :] = r[ii].astype(BF16)
                yield [r[4][:8], r[4][8:]]
            return _Piece(emit, [(38, 6)], deadline, release)

        when = {}
        for jj in JJ_ORDER:
            first = uses(lambda j, q: j[0] == unit and g in j[1] and q == jj)[0]
            prev = -1 if unit < 2 else uses(
                lambda j, q: j[0] == unit - 2 and g in j[1] and q == jj)[1]
            when[jj] = first if first in FENCES else first - MARGIN, prev
        if idx in BY_COLUMN:
            return [row(h) for h in range(64)] + [
                col(th, jj, *when[jj]) for jj in JJ_ORDER for th in range(16)]
        out = [row(h) for h in range(6)]
        if unit >= 2:
            out[0].release = {2: 216, 3: 360}[unit] - MARGIN
        for th in range(16):
            out += [col(th, jj, *when[jj]) for jj in JJ_ORDER]
            out += [row(h) for h in range(4 * th + 6, min(64, 4 * th + 10))]
        return out

    def out_stage(idx):
        unit, g = idx // 4, idx % 4
        bg = idx % 8
        last = uses(lambda j, q: j[0] == unit and g in j[2])[1]
        mb = idx % 8
        deadline = (216, 360)[unit] - 5 * (3 - g) if unit < 2 else out_block[bg]

        def rows(th, e, z):
            r = pl.ds(th * 16 + e * 8, 8)
            for i in range(6):
                z.append(_out_tf(*[ms[mb, i * 6 + j, r, :] for j in range(6)]))
                yield [z[-1][3]]

        def pixels(z, q):
            y = _out_tf(*[z[i][q] for i in range(6)])
            return [_mul(y[p], PA ** (p + q - 3)) for p in range(4)]

        def hidden(th, e):
            def emit():
                z = []
                yield from rows(th, e, z)
                acc = [acc_s[idx + 8, 0], acc_s[idx + 8, 1]] if th or e else [None, None]
                for q in range(4):
                    y = pixels(z, q)
                    for p in range(4):
                        hs[bg, 4 * th + p, q, pl.ds(e * 8, 8), :] = y[p]
                    sq = [lax.mul(v, v) for v in y]
                    for i, v in enumerate((y, sq)):
                        v = _add(_add(v[0], v[1]), _add(v[2], v[3]))
                        acc[i] = v if acc[i] is None else _add(acc[i], v)
                    if q == 3:
                        acc[0] = lax.select(ts[0, 0, 0:8, :] == 0.0, acc[0], acc[1])
                        acc_s[idx + 8, 0], acc_s[idx + 8, 1] = acc
                    yield acc[:1] if q == 3 else acc[1:]
            return _Piece(emit, [(14, 0)] * 6 + [(29, 4.5)] * 4, deadline, last)

        def residual(th, e, p, kq):
            w = xw[bg, th, p, pl.ds(2 * e + kq, 8, stride=4), :]
            return _lo(w), _hi(w)

        def put(th, e, p, kq, lo, hi):
            v = lax.bitcast_convert_type(_cat(lo, hi).astype(BF16).astype(F32), U32)
            v = lax.bitwise_or(lax.shift_right_logical(v[:8], np.uint32(16)), v[8:])
            ow[bg, th, p, pl.ds(2 * e + kq, 8, stride=4), :] = v
            return v

        def closing(phase, th, e):
            r, half = pl.ds(th * 16 + e * 8, 8), pl.ds(e * 8, 8)

            def line(i):
                return _out_tf(*[ms[mb, i * 6 + j, r, :] for j in range(6)])

            def scale(v, p, q, f=1.0):
                return _mul(v, f * PA ** (p + q - 3))

            def emit():
                if phase < 2:
                    z1 = line(2 * phase + 1)
                    yield [z1[3]]
                    z2 = line(2 * phase + 2)
                    yield [z2[3]]
                    sd = [(_add(u, v), _sub(u, v)) for u, v in zip(z1, z2)]
                    for p in range(4):
                        if phase == 0:
                            x = residual(th, e, p, 0) + residual(th, e, p, 1)
                            y = [_add(scale(sd[q][p % 2], p, q), x[q]) for q in range(4)]
                        else:
                            y = [_sub(ts[4 * th + p + 1, q, half, :],
                                      scale(sd[q][p % 2], p, q, PA ** (4 - 2 * p)))
                                 for q in range(4)]
                        if phase == 1 and p in (1, 2):
                            y = [put(th, e, p, kq, *y[2 * kq:2 * kq + 2]) for kq in range(2)]
                        else:
                            for q in range(4):
                                ts[4 * th + p + 1, q, half, :] = y[q]
                        yield y[-1:]
                else:
                    p = 3 * (phase - 2)
                    z = line(5 * (phase - 2))
                    y = [_add(ts[4 * th + p + 1, q, half, :], scale(z[q], p, q))
                         for q in range(4)]
                    yield [put(th, e, p, kq, *y[2 * kq:2 * kq + 2]) for kq in range(2)]

            costs = ([(14, 0)] * 2 + [(14, 4)] * 4, [(14, 0)] * 2 + [(17, 3)] * 4,
                     [(35, 2)], [(35, 2)])[phase]
            return _Piece(emit, costs, (571, 571, 574, NMM + 1)[phase],
                          NMM - 1 - (24, 12, 6, 0)[phase] - (phase > 0))

        def final(th, e):
            def emit():
                z = []
                yield from rows(th, e, z)
                for kq in range(2):
                    y0 = pixels(z, 2 * kq)
                    yield [y0[3]]
                    y1 = pixels(z, 2 * kq + 1)
                    yield [y1[3]]
                    for p in range(4):
                        lo, hi = residual(th, e, p, kq)
                        yield [put(th, e, p, kq, _add(y0[p], lo), _add(y1[p], hi))]
            return _Piece(emit, [(14, 0)] * 6 + ([(18, 0)] * 2 + [(11, 1)] * 4) * 2, deadline, last)

        if unit < 2:
            fin = finalize(idx + 8)
            fin.after = emb_stream[-1]
            fin.deadline = deadline
            return [hidden(th, e) for th in range(16) for e in range(2)] + [fin]
        if idx == 15:
            return [closing(n, th, e) for n in range(4) for th in range(16) for e in range(2)]
        return [final(th, e) for th in range(16) for e in range(2)]

    def w_stage(c, n, k, phases):
        def piece(r, jjs):
            def emit():
                def out(jj, t):
                    u = _w_tf(*t)
                    for ii in range(6):
                        us[u_slot(c, n), ii * 6 + jj, k, pl.ds(r * 16, 16), :] = u[ii].astype(BF16)
                    return [u[i][h:h + 8] for i in ((2, 4) if jj in (0, 5) else (4,))
                            for h in (0, 8)]

                def tap(j):
                    return [ws[c, k if jjs[0] in (0, 5) else k + zero * jjs[0],
                               i, j, pl.ds(128 * n + 16 * r, 16), :].astype(F32)
                            for i in range(3)]

                def scaled(g, f):
                    return [_mul(g[i], W_SCALE * PA ** i * f) for i in range(3)]

                g = {j: tap(j) for j in {(0,): (0,), (5,): (2,)}.get(jjs, (0, 2, 1))}
                if 0 in jjs:
                    yield out(0, scaled(g[0], NA))
                if 5 in jjs:
                    yield out(5, scaled(g[2], NA / PA ** 4))
                if len(jjs) == 2:
                    g = [scaled(g[j], (PA if 1 in jjs else PB) ** j) for j in range(3)]
                    e = [_add(*v) for v in zip(g[0], g[2])]
                    yield out(jjs[0], [_add(*v) for v in zip(e, g[1])])
                    yield out(jjs[1], [_sub(*v) for v in zip(e, g[1])])
                elif len(jjs) == 6:
                    g = [scaled(g[j], PA ** j) for j in range(3)]
                    e = [_add(u, _mul(v, PB ** 4)) for u, v in zip(g[0], g[2])]
                    o = [_mul(v, PB * PB) for v in g[1]]
                    yield out(3, [_add(*v) for v in zip(e, o)])
                    yield out(4, [_sub(*v) for v in zip(e, o)])
                    e = [_add(*v) for v in zip(g[0], g[2])]
                    yield out(1, [_add(*v) for v in zip(e, g[1])])
                    yield out(2, [_sub(*v) for v in zip(e, g[1])])
            return emit

        res = []
        for jjs in phases:
            first = uses(lambda j, q: j[0] // 2 == c and k in j[1] and n in j[2] and q in jjs)[0]
            prev = -1 if c == 0 or n == 0 else 288 - MARGIN
            prev = max(prev, w_ready[4 * c + k])
            costs = {1: [42], 2: [76, 34], 6: [42, 42, 76, 34, 40, 34]}[len(jjs)]
            costs = [(v, 6) for v in costs]
            res += [_Piece(piece(r, jjs), costs,
                           first if first in FENCES else first - MARGIN - 1, prev) for r in range(8)]
        return res

    def emb_part(e, release):
        def emit():
            t = tv[:, pl.ds(128 * e, 128)].astype(F32)
            t = (t * jax.nn.sigmoid(t)).astype(BF16)
            v = jnp.dot(t, wes[pl.ds(128 * e, 128), :], preferred_element_type=F32)
            emb_s[...] = emb_s[...] + v if e else v
            yield []
        return _Piece(emit, [(20, 4)], release + 2, release)

    fences = {
        10: [x_copy(1)],
        24: [w_copy(0, 1)],
        46: [x_copy(2), w_copy(0, 2), x_copy(3)],
        89: [w_copy(0, 3), x_copy(4), x_copy(5)],
        144: [x_copy(6), x_copy(7), *p_copy[2:]],
        216: [w_copy(1, k) for k in ALL],
    }
    starts = {10: fences[24] + fences[46][:1], 24: fences[46][1:], 46: fences[89],
              89: [x_copy(6), x_copy(7), p_copy[5]], 144: fences[216],
              503: [o_copy(bg) for bg in range(5)], 555: [o_copy(5), o_copy(6)],
              571: [o_copy(7, 1), o_copy(7, 2)], 574: [o_copy(7, 0)]}
    x_ready = [f - MARGIN for f in (1, 10, 46, 46, 89, 89, 144, 144)]
    w_ready = [f - MARGIN for f in (1, 24, 46, 89, 216, 216, 216, 216)]
    out_block = (499, 500, 501, 502, 503, 554, 555, None)
    emb_stream = [emb_part(e, 146 + 2 * e) for e in range(9)]
    stat_streams = [x_stats(bg) for bg in range(8)] + [out_stage(i) for i in range(8)]
    for bg in range(8):
        stat_streams[bg][0].release = x_ready[bg]
    in_stream = []
    for idx in range(16):
        in_stream += in_stage(idx, stat_streams[idx][-1])
        if idx == 0:
            for p in in_stream[:100]:
                p.deadline = 0
            in_stream.insert(100, waiting(w_copy(0, 0)))
            w_landed = in_stream[100]
    split, whole = ((0,), (5,), (1, 2), (3, 4)), (JJ_ORDER,)
    w_stream = []
    for k in ALL:
        for jjs in split:
            for n in ALL:
                w_stream += w_stage(0, n, k, (jjs,))
    w_stream[0].after = w_landed
    for n in ALL:
        for k in ALL:
            w_stream += w_stage(1, n, k, whole)
    plan = _plan(stat_streams + [in_stream, w_stream, emb_stream]
                 + [out_stage(i) for i in range(8, 16)])

    running = {}

    def advance(slot):
        pend = []
        for p in plan[slot + 1]:
            if id(p) not in running:
                running[id(p)] = p.emit()
            pend += next(running[id(p)])
        return pend

    def matmuls(lo, hi, zero):
        keeps = [ts[0, i, 0:8, :] == 0.0 for i in range(4)]
        for mm in range(lo, hi):
            s, t = divmod(mm, 36)
            unit, ks, ns, acc = JOBS[s]
            ij = (t % 6) * 6 + JJ_ORDER[t // 6]
            if s == len(JOBS) - 1:
                ij = (1, 2, 3, 4, 0, 5)[t // 6] * 6 + t % 6
            blocks = [[] for _ in ks]
            src = ij if s < 6 or 36 * s <= lo else ij + zero * (s % 4)
            whole = [vw[unit % 2][src, k] for k in ks]
            for r in range(16):
                pend = advance(16 * mm + r)
                w = [lax.slice(v, (8 * r, 0), (8 * r + 8, 128)) for v in whole]
                for i, a in enumerate(pend[-4 * len(ks):]):
                    w[i % len(ks)] = lax.select(
                        keeps[i // len(ks)], w[i % len(ks)], lax.bitcast_convert_type(a, U32))
                for b, v in zip(blocks, w):
                    b.append(v)
            lhs = lax.concatenate(
                [pltpu.bitcast(lax.concatenate(b, 0), BF16) for b in blocks], 1)
            rhs = lax.concatenate([lax.concatenate(
                [pltpu.bitcast(uw[u_slot(unit // 2, n), ij, k], BF16) for k in ks], 1) for n in ns], 0)
            res = lax.dot_general(lhs, rhs, (((1,), (1,)), ((), ())),
                                  preferred_element_type=F32)
            for i, n in enumerate(ns):
                mb = unit % 2 * 4 + n
                v = res[:, 128 * i:128 * (i + 1)]
                ms[mb, ij] = _add(ms[mb, ij], v) if acc else v
            latest[:] = [v[:8]] if mm + 1 < hi else []
        if hi == NMM:
            advance(16 * NMM)

    for cp in p_copy[:5]:
        cp.start()
    for n in range(4):
        x_copy(0, n).start()
    w_copy(0, 0).start()
    ts[0] = jnp.zeros((6, 16, 128), F32)
    ts[65] = jnp.zeros((6, 16, 128), F32)
    zero = lax.fori_loop(0, 3, lambda i, c: c + i, 0) - 3

    advance(-1)
    for lo, hi in zip((0,) + FENCES, FENCES + (NMM,)):
        for cp in fences.get(lo, ()):
            cp.wait()
        for cp in starts.get(lo, ()):
            cp.start()
        pl.when(zero <= lo)(lambda: matmuls(lo, hi, zero))
    o_copy(7, 3).start()
    for bg in range(7):
        o_copy(bg).wait()
    for n in range(4):
        o_copy(7, n).wait()


@jax.jit
def pallas_standalone__adm_resblock__diffusion_kernel(
        x, t_emb, g1, be1, w1, w_emb, g2, be2, w2):
    B, C, H, W = x.shape
    E = t_emb.shape[1]
    assert (B, C, H, W, E) == (2, 512, 64, 64, 1152)
    xt = x.transpose(0, 2, 3, 1).reshape(B, H // 4, 4, W, C)
    hbm = pl.BlockSpec(memory_space=pl.ANY)
    out = pl.pallas_call(
        _kernel,
        out_shape=jax.ShapeDtypeStruct(xt.shape, x.dtype),
        in_specs=[hbm] * 9,
        out_specs=hbm,
        scratch_shapes=[
            pltpu.VMEM((9, 16, 4, W, 128), BF16),
            pltpu.VMEM((8, 16, 4, W, 128), BF16),
            pltpu.VMEM((2, 4, 3, 3, 512, 128), BF16),
            pltpu.VMEM((E, C), BF16),
            pltpu.VMEM((B, E), BF16),
            [pltpu.VMEM((C,), BF16)] * 4,
            pltpu.VMEM((5, 36, 4, 128, 128), BF16),
            pltpu.VMEM((36, 4, 256, 128), BF16),
            pltpu.VMEM((36, 4, 256, 128), BF16),
            pltpu.VMEM((8, 36, 256, 128), F32),
            pltpu.VMEM((8, 64, 4, 16, 128), F32),
            pltpu.VMEM((66, 6, 16, 128), F32),
            pltpu.VMEM((B, C), F32),
            pltpu.VMEM((16, 2, 8, 128), F32),
            pltpu.VMEM((16, 2, 8, 128), F32),
            pltpu.SemaphoreType.DMA((12,)),
            pltpu.SemaphoreType.DMA((8,)),
            pltpu.SemaphoreType.DMA((6,)),
            pltpu.SemaphoreType.DMA((12,)),
        ],
        compiler_params=pltpu.CompilerParams(vmem_limit_bytes=126 * 2 ** 20),
        name="resblock",
    )(xt, t_emb, g1, be1, w1.transpose(2, 3, 0, 1), w_emb, g2, be2, w2.transpose(2, 3, 0, 1))
    return out.reshape(B, H, W, C).transpose(0, 3, 1, 2)
```

```python
import jax
import jax.numpy as jnp
import numpy as np
from jax import lax
import jax.experimental.pallas as pl
import jax.experimental.pallas.tpu as pltpu

F32, BF16, U32 = jnp.float32, jnp.bfloat16, jnp.uint32

PA, PB = 1.5, 2.0 / 3.0
NA = 2.0 * PA * PA * (PA * PA - PB * PB)
EPS = 1e-5

JJ_ORDER = (0, 5, 1, 2, 3, 4)
ALL = (0, 1, 2, 3)
JOBS = (
    (0, (0,), ALL, False), (0, (1,), ALL, True), (0, (2,), ALL, True), (0, (3,), ALL, True),
    (1, (0, 1), (0, 1), False), (1, (0, 1), (2, 3), False),
    (1, (2, 3), (0, 1), True), (1, (2, 3), (2, 3), True),
    (2, ALL, (0,), False), (2, ALL, (1,), False), (2, ALL, (2,), False), (2, ALL, (3,), False),
    (3, ALL, (0,), False), (3, ALL, (1,), False), (3, ALL, (2,), False), (3, ALL, (3,), False),
)
FENCES = (4, 13, 25, 47, 89, 144, 180, 216, 288, 360, 503, 555, 571, 574)
BY_COLUMN = (0, 4, 5, 7)
NMM = 36 * len(JOBS)
MARGIN = 2
LATENCY = 2
STREAM_RATE = 600
STORE_RATE = 139
ALU0 = 48
ALU1 = 46
ALU2 = 43
ALU3 = 40
ALU_RATE = (ALU0,) * 4 + (ALU1,) * 4 + (ALU2,) * 4 + (ALU3,) * 4


def u_slot(c, n):
    return (4 * c + n) % 5


_add, _sub = lax.add, lax.sub


def _mul(x, c):
    return x if abs(c - 1.0) < 1e-12 else lax.mul(x, np.float32(c))


IN_SCALE = (PA, PA * PA, PB, 1.0)
W_SCALE = PA ** 3 / NA ** 2


def _in_tf(d0, d1, d2, d3, d4, d5):
    p = _mul(d2, PB ** 4)
    ea, eb = _sub(d4, p), _sub(d4, d2)
    r0 = _add(_sub(d0, p), eb)
    t = _mul(d3, PA ** 4)
    oa, ob = _mul(_sub(t, d1), PB * PB), _sub(d3, d1)
    r5 = _sub(_sub(d5, t), ob)
    return r0, _add(ea, oa), _sub(ea, oa), _add(eb, ob), _sub(eb, ob), r5


def _out_tf(m0, m1, m2, m3, m4, m5):
    sa, da = _add(m1, m2), _sub(m1, m2)
    sb, db = _add(m3, m4), _sub(m3, m4)
    y0 = _sub(_add(m0, sa), _mul(sb, PA ** 4))
    y1 = _sub(da, _mul(db, PA * PA))
    y2 = _sub(sa, sb)
    y3 = _add(_sub(da, _mul(db, PB * PB)), m5)
    return y0, y1, y2, y3


def _w_tf(g0, g1, g2):
    ea = _add(g0, g2)
    eb, ob = _add(g0, _mul(g2, PB ** 4)), _mul(g1, PB * PB)
    return (_mul(g0, NA), _add(ea, g1), _sub(ea, g1), _add(eb, ob), _sub(eb, ob),
            _mul(g2, NA / PA ** 6))


def _lo(w):
    return lax.bitcast_convert_type(lax.shift_left(w, np.uint32(16)), F32)


def _hi(w):
    return lax.bitcast_convert_type(lax.bitwise_and(w, np.uint32(0xFFFF0000)), F32)


def _cat(a, b):
    return lax.concatenate([a, b], 0)


class _Piece:
    def __init__(self, emit, costs, deadline, release=-1, after=None):
        self.emit, self.costs = emit, np.array(costs, float)
        self.deadline = deadline
        self.release = release
        self.after = after
        self.time, self.gap = None, False


def _plan(streams):
    for st in streams:
        for p in st:
            p.soft = float(p.deadline)
    for _ in range(4):
        for st in streams:
            for i in reversed(range(len(st))):
                p = st[i]
                start = p.soft - p.costs[:, 0].sum() / STREAM_RATE
                if i:
                    st[i - 1].deadline = min(st[i - 1].deadline, p.deadline)
                    st[i - 1].soft = min(st[i - 1].soft, start)
                if p.after is not None:
                    p.after.deadline = min(p.after.deadline, p.deadline)
                    p.after.soft = min(p.after.soft, start - LATENCY)
    pos = [0] * len(streams)
    plan = [[] for _ in range(16 * NMM + 2)]
    cur, credit, rate = None, np.zeros(2), np.zeros(2)

    def pick(mm):
        best = None
        for i, st in enumerate(streams):
            if pos[i] == len(st):
                continue
            p = st[pos[i]]
            urgent = p.deadline <= max(mm, 0) + (left == 0) or mm > NMM
            if not urgent and (mm < 0 or p.release + MARGIN > mm):
                continue
            if p.gap and not urgent and st[pos[i] - 1].time in (None, mm, mm - 1):
                continue
            if p.after is not None and (p.after.time is None or (
                    not urgent and p.after.time + LATENCY > mm)):
                continue
            key = (not urgent, credit[1] <= 0 and p.costs[:, 1].any(), p.soft)
            if best is None or key < best[0]:
                best = key, i
        return best

    def affordable(cost):
        return all(c > 0 or not need for c, need in zip(credit, cost))

    for slot in range(-1, 16 * NMM + 1):
        mm = slot // 16 if slot < 16 * NMM else NMM + 1
        if 0 <= mm < NMM:
            _, ks, ns, acc = JOBS[mm // 36]
            rate = np.array([ALU_RATE[mm // 36] - 2 * len(ns) * (len(ks) - (not acc)),
                             STORE_RATE / 10 - 2 * len(ns)])
            credit = np.minimum(credit + rate, 2 * rate)
        left = min([16 * f - 1 - slot for f in FENCES if 16 * f > slot], default=1000)
        while True:
            best = pick(mm)
            if cur is None:
                if best is None:
                    break
                i = best[1]
                p = streams[i][pos[i]]
                if best[0][0] and not (affordable(p.costs.sum(0)) and all(
                        p.costs.sum(0) <= credit + left * rate)):
                    break
                assert p.release < max(mm, 0) and (mm < p.deadline or mm not in FENCES)
                pos[i] += 1
                cur = [p, 0]
            p, k = cur
            if not affordable(p.costs[k]) and left and p.deadline > max(mm, 0) and (
                    mm <= NMM and (best is None or best[0][0])):
                break
            plan[slot + 1].append(p)
            credit = np.maximum(credit - p.costs[k], -2 * rate)
            cur[1] += 1
            if cur[1] == len(p.costs):
                p.time, cur = mm, None
    assert all(n == len(st) for n, st in zip(pos, streams))
    return plan


def _kernel(x_hbm, t_hbm, g1_hbm, be1_hbm, w1_hbm, we_hbm, g2_hbm, be2_hbm, w2_hbm,
            o_hbm,
            xs, ws, wes, tv, gv, us, v0, v1, ms, hs, ts, emb_s, acc_s, cf,
            xsem, wsem, psem, osem):
    xw = xs.bitcast(U32)
    uw = us.bitcast(U32)
    vs = (v0, v1)
    vw = (v0.bitcast(U32), v1.bitcast(U32))

    def x_copy(bg, part=None):
        rows = slice(None) if part is None else pl.ds(4 * part, 4)
        return pltpu.make_async_copy(
            x_hbm.at[bg // 4, rows, :, :, pl.ds(bg % 4 * 128, 128)], xs.at[bg, rows],
            xsem.at[bg if part is None else 8 + part])

    def w_copy(c, k, j=None):
        cols = slice(None) if j is None else pl.ds(j, 1)
        return pltpu.make_async_copy(
            (w1_hbm, w2_hbm)[c].at[:, cols, :, pl.ds(k * 128, 128)], ws.at[c, k, :, cols],
            wsem.at[4 * c + k if j is None else 8 + j])

    def o_copy(bg, part=None):
        rows = slice(None) if part is None else pl.ds(part, 1)
        return pltpu.make_async_copy(
            xs.at[bg, :, rows], o_hbm.at[bg // 4, :, rows, :, pl.ds(bg % 4 * 128, 128)],
            osem.at[bg if part is None else 8 + part])

    p_copy = [pltpu.make_async_copy(src, dst, psem.at[i]) for i, (src, dst) in enumerate(
        ((g1_hbm, gv[0]), (be1_hbm, gv[1]), (g2_hbm, gv[2]), (be2_hbm, gv[3]),
         (t_hbm, tv), (we_hbm, wes)))]

    def start_rest():
        for cp in fences[13]:
            cp.start()
        yield []

    def waiting(*copies):
        def emit():
            for cp in copies:
                cp.wait()
            yield []
        return _Piece(emit, [(1, 0)], NMM + 1)

    def uses(pred):
        t = [36 * s + 6 * n + ii for s, job in enumerate(JOBS)
             for n, jj in enumerate(JJ_ORDER) for ii in range(6) if pred(job, jj)]
        return min(t), max(t)

    def finalize(idx):
        def emit():
            coefficients(idx)
            yield []
        fin = _Piece(emit, [(30, 0)], NMM + 1)
        fin.gap = True
        return fin

    def coefficients(idx):
        g = idx % 4
        s1, s2 = acc_s[idx, 0], acc_s[idx, 1]
        emb = emb_s[pl.ds(idx // 4 - 2, 1), pl.ds(128 * g, 128)] if idx >= 8 else None
        gamma, beta = (r[...].astype(F32).reshape(1, 512)[:, 128 * g:128 * (g + 1)]
                       for r in gv[idx // 8 * 2:idx // 8 * 2 + 2])
        m, q = s1 * (1.0 / 4096.0), s2 * (1.0 / 4096.0)
        if emb is not None:
            m, q = m + emb * 0.125, q + emb * (2.0 * m + emb * 0.125)
        v = _cat(m, q) * (1.0 / 128.0)
        if idx == 0:
            v = jnp.sum(v, axis=1, keepdims=True)
        else:
            parts = []
            for _ in range(4):
                parts.append(v.astype(BF16))
                v = v - parts[-1].astype(F32)
            v = jnp.dot(lax.concatenate(parts, 1), jnp.ones((512, 128), BF16),
                        preferred_element_type=F32)
        mu = jnp.sum(v[:8], axis=0, keepdims=True)
        var = jnp.maximum(jnp.sum(v[8:], axis=0, keepdims=True) - mu * mu, 0.0)
        sc = lax.rsqrt(var + EPS) * gamma * 0.5
        sh = (0.5 * beta) - (mu if emb is None else mu - emb) * sc
        cf[idx, 0] = jnp.broadcast_to(sc, (8, 128))
        cf[idx, 1] = jnp.broadcast_to(sh, (8, 128))

    def x_stats(bg):
        def part(n):
            def emit():
                acc = [acc_s[bg, 0], acc_s[bg, 1]] if n else [None, None]
                for r in range(8 * n, 8 * n + 8):
                    w = xw[bg, r // 4, r % 4]
                    lo, hi = _lo(w), _hi(w)
                    a = _add(lo, hi)
                    q = _add(lax.mul(lo, lo), lax.mul(hi, hi))
                    for i, v in enumerate((a, q)):
                        v = _add(v[:16], v[16:])
                        v = _add(v[:8], v[8:])
                        acc[i] = v if acc[i] is None else _add(acc[i], v)
                    if r % 8 == 7:
                        acc_s[bg, 0], acc_s[bg, 1] = acc
                    yield list(acc)
            return _Piece(emit, [(34, 0)] * 8, NMM + 1)

        out = []
        for n in range(8):
            if bg == 0 and n % 2 == 0:
                out.append(waiting(x_copy(0, n // 2)))
            out.append(part(n))
        if bg == 0:
            out += [waiting(*p_copy[:2]), _Piece(start_rest, [(1, 0)], NMM + 1)]
        return out + [finalize(bg)]

    def in_stage(idx, stats):
        unit, g = idx // 4, idx % 4

        def row(h):
            def emit():
                sc, sh = cf[idx, 0], cf[idx, 1]
                sc, sh = _cat(sc, sc), _cat(sh, sh)
                if idx < 8:
                    w = [xw[idx, h // 4, h % 4, pl.ds(k, 8, stride=4), :] for k in range(4)]
                    w02, w13 = _cat(w[0], w[2]), _cat(w[1], w[3])
                    y = [_lo(w02), _hi(w02), _lo(w13), _hi(w13)]
                else:
                    y = [hs[idx - 8, h, j] for j in range(4)]
                a = []
                for j, yj in enumerate(y):
                    u = _add(lax.mul(yj, sc), sh)
                    v = _mul(u, IN_SCALE[h % 4] * IN_SCALE[j])
                    a.append(_add(v, lax.mul(v, lax.tanh(u))))
                yield [a[3][8:]]
                sub = lax.broadcasted_iota(jnp.int32, (8, 128), 0)
                pad = jnp.zeros((8, 128), F32)
                left = lax.select(sub == 0, pad, pltpu.roll(a[3][8:], 1, 0))
                right = lax.select(sub == 7, pad, pltpu.roll(a[0][:8], 7, 0))
                r = _in_tf(_cat(left, a[3][:8]), a[0], a[1], a[2], a[3], _cat(a[0][8:], right))
                for jj in range(6):
                    ts[h + 1, jj] = r[jj]
                yield [r[4][:8], r[4][8:]]
            return _Piece(emit, [(47 if idx < 8 else 39, 0), (36, 12)], NMM + 1, after=stats)

        def col(th, jj, deadline, release):
            def emit():
                r = _in_tf(*[ts[4 * th + i, jj] for i in range(6)])
                for ii in range(6):
                    vs[unit % 2][ii * 6 + jj, g, pl.ds(th * 16, 16), :] = r[ii].astype(BF16)
                yield [r[4][:8], r[4][8:]]
            return _Piece(emit, [(38, 6)], deadline, release)

        when = {}
        for jj in JJ_ORDER:
            first = uses(lambda j, q: j[0] == unit and g in j[1] and q == jj)[0]
            prev = -1 if unit < 2 else uses(
                lambda j, q: j[0] == unit - 2 and g in j[1] and q == jj)[1]
            when[jj] = first if first in FENCES else first - MARGIN, prev
        if idx in BY_COLUMN:
            rows = [row(h) for h in range(64)]
            if idx == 7:
                rows[-1].deadline = 190
            return rows + [
                col(th, jj, *when[jj]) for jj in JJ_ORDER for th in range(16)]
        out = [row(h) for h in range(6)]
        if unit >= 2:
            out[0].release = {2: 216, 3: 360}[unit] - MARGIN
        for th in range(16):
            out += [col(th, jj, *when[jj]) for jj in JJ_ORDER]
            out += [row(h) for h in range(4 * th + 6, min(64, 4 * th + 10))]
        return out

    def out_stage(idx):
        unit, g = idx // 4, idx % 4
        bg = idx % 8
        last = uses(lambda j, q: j[0] == unit and g in j[2])[1]
        mb = idx % 8
        deadline = (216, 360)[unit] - 3 * (3 - g) if unit < 2 else out_block[bg]

        def rows(th, e, z):
            r = pl.ds(th * 16 + e * 8, 8)
            for i in range(6):
                z.append(_out_tf(*[ms[mb, i * 6 + j, r, :] for j in range(6)]))
                yield [z[-1][3]]

        def pixels(z, q):
            y = _out_tf(*[z[i][q] for i in range(6)])
            return [_mul(y[p], PA ** (p + q - 3)) for p in range(4)]

        def hidden(th, e):
            def emit():
                z = []
                yield from rows(th, e, z)
                acc = [acc_s[idx + 8, 0], acc_s[idx + 8, 1]] if th or e else [None, None]
                for q in range(4):
                    y = pixels(z, q)
                    for p in range(4):
                        hs[bg, 4 * th + p, q, pl.ds(e * 8, 8), :] = y[p]
                    sq = [lax.mul(v, v) for v in y]
                    for i, v in enumerate((y, sq)):
                        v = _add(_add(v[0], v[1]), _add(v[2], v[3]))
                        acc[i] = v if acc[i] is None else _add(acc[i], v)
                    if q == 3:
                        acc_s[idx + 8, 0], acc_s[idx + 8, 1] = acc
                    yield list(acc) if q == 3 else acc[1:]
            return _Piece(emit, [(14, 0)] * 6 + [(29, 4.5)] * 4, deadline, last)

        def residual(th, e, p, kq):
            w = xw[bg, th, p, pl.ds(2 * e + kq, 8, stride=4), :]
            return _lo(w), _hi(w)

        def put(th, e, p, kq, lo, hi):
            v = lax.bitcast_convert_type(_cat(lo, hi).astype(BF16).astype(F32), U32)
            v = lax.bitwise_or(lax.shift_right_logical(v[:8], np.uint32(16)), v[8:])
            xw[bg, th, p, pl.ds(2 * e + kq, 8, stride=4), :] = v
            return v

        def closing(phase, th, e):
            r, half = pl.ds(th * 16 + e * 8, 8), pl.ds(e * 8, 8)

            def line(i):
                return _out_tf(*[ms[mb, i * 6 + j, r, :] for j in range(6)])

            def scale(v, p, q, f=1.0):
                return _mul(v, f * PA ** (p + q - 3))

            def emit():
                if phase < 2:
                    z1 = line(2 * phase + 1)
                    yield [z1[3]]
                    z2 = line(2 * phase + 2)
                    yield [z2[3]]
                    sd = [(_add(u, v), _sub(u, v)) for u, v in zip(z1, z2)]
                    for p in range(4):
                        if phase == 0:
                            x = residual(th, e, p, 0) + residual(th, e, p, 1)
                            y = [_add(scale(sd[q][p % 2], p, q), x[q]) for q in range(4)]
                        else:
                            y = [_sub(ts[4 * th + p + 1, q, half, :],
                                      scale(sd[q][p % 2], p, q, PA ** (4 - 2 * p)))
                                 for q in range(4)]
                        if phase == 1 and p in (1, 2):
                            y = [put(th, e, p, kq, *y[2 * kq:2 * kq + 2]) for kq in range(2)]
                        else:
                            for q in range(4):
                                ts[4 * th + p + 1, q, half, :] = y[q]
                        yield y[-1:]
                else:
                    p = 3 * (phase - 2)
                    z = line(5 * (phase - 2))
                    y = [_add(ts[4 * th + p + 1, q, half, :], scale(z[q], p, q))
                         for q in range(4)]
                    yield [put(th, e, p, kq, *y[2 * kq:2 * kq + 2]) for kq in range(2)]

            costs = ([(14, 0)] * 2 + [(14, 4)] * 4, [(14, 0)] * 2 + [(17, 3)] * 4,
                     [(35, 2)], [(35, 2)])[phase]
            return _Piece(emit, costs, (571, 571, 574, NMM + 1)[phase],
                          NMM - 1 - (24, 12, 6, 0)[phase] - (phase > 0))

        def final(th, e):
            def emit():
                z = []
                yield from rows(th, e, z)
                for kq in range(2):
                    y0 = pixels(z, 2 * kq)
                    yield [y0[3]]
                    y1 = pixels(z, 2 * kq + 1)
                    yield [y1[3]]
                    for p in range(4):
                        lo, hi = residual(th, e, p, kq)
                        yield [put(th, e, p, kq, _add(y0[p], lo), _add(y1[p], hi))]
            return _Piece(emit, [(14, 0)] * 6 + ([(18, 0)] * 2 + [(11, 1)] * 4) * 2, deadline, last)

        if unit < 2:
            fin = finalize(idx + 8)
            fin.after = emb_stream[-1]
            fin.deadline = deadline
            return [hidden(th, e) for th in range(16) for e in range(2)] + [fin]
        if idx == 15:
            return [closing(n, th, e) for n in range(4) for th in range(16) for e in range(2)]
        return [final(th, e) for th in range(16) for e in range(2)]

    def w_stage(c, n, k, phases):
        def piece(r, jjs):
            def emit():
                def out(jj, t):
                    u = _w_tf(*t)
                    for ii in range(6):
                        us[u_slot(c, n), ii * 6 + jj, k, pl.ds(r * 16, 16), :] = u[ii].astype(BF16)
                    return [u[i][h:h + 8] for i in ((2, 4) if jj in (0, 5) else (4,))
                            for h in (0, 8)]

                def tap(j):
                    return [ws[c, k if jjs[0] in (0, 5) else k + zero * jjs[0],
                               i, j, pl.ds(128 * n + 16 * r, 16), :].astype(F32)
                            for i in range(3)]

                def scaled(g, f):
                    return [_mul(g[i], W_SCALE * PA ** i * f) for i in range(3)]

                g = {j: tap(j) for j in {(0,): (0,), (5,): (2,)}.get(jjs, (0, 2, 1))}
                if 0 in jjs:
                    yield out(0, scaled(g[0], NA))
                if 5 in jjs:
                    yield out(5, scaled(g[2], NA / PA ** 4))
                if len(jjs) == 2:
                    g = [scaled(g[j], (PA if 1 in jjs else PB) ** j) for j in range(3)]
                    e = [_add(*v) for v in zip(g[0], g[2])]
                    yield out(jjs[0], [_add(*v) for v in zip(e, g[1])])
                    yield out(jjs[1], [_sub(*v) for v in zip(e, g[1])])
                elif len(jjs) == 6:
                    g = [scaled(g[j], PA ** j) for j in range(3)]
                    e = [_add(u, _mul(v, PB ** 4)) for u, v in zip(g[0], g[2])]
                    o = [_mul(v, PB * PB) for v in g[1]]
                    yield out(3, [_add(*v) for v in zip(e, o)])
                    yield out(4, [_sub(*v) for v in zip(e, o)])
                    e = [_add(*v) for v in zip(g[0], g[2])]
                    yield out(1, [_add(*v) for v in zip(e, g[1])])
                    yield out(2, [_sub(*v) for v in zip(e, g[1])])
            return emit

        res = []
        for jjs in phases:
            first = uses(lambda j, q: j[0] // 2 == c and k in j[1] and n in j[2] and q in jjs)[0]
            prev = 288 - MARGIN if c and n else -1
            if (c, k, jjs) != (0, 0, (0,)):
                prev = max(prev, w_ready[4 * c + k])
            costs = {1: [42], 2: [76, 34], 6: [42, 42, 76, 34, 40, 34]}[len(jjs)]
            costs = [(v, 6) for v in costs]
            res += [_Piece(piece(r, jjs), costs,
                           first if first in FENCES else first - (1 if first < 13 else 3), prev) for r in range(8)]
        return res

    def emb_part(e, release):
        def emit():
            t = tv[:, pl.ds(128 * e, 128)].astype(F32)
            t = (t * jax.nn.sigmoid(t)).astype(BF16)
            v = jnp.dot(t, wes[pl.ds(128 * e, 128), :], preferred_element_type=F32)
            emb_s[...] = emb_s[...] + v if e else v
            yield []
        return _Piece(emit, [(20, 4)], release + 5, release)

    fences = {
        4: [w_copy(0, 0, 2), w_copy(0, 0, 1)],
        13: [x_copy(1)],
        25: [w_copy(0, 1)],
        47: [x_copy(2), w_copy(0, 2), x_copy(3)],
        89: [w_copy(0, 3), x_copy(4), x_copy(5)],
        144: [x_copy(6), x_copy(7), *p_copy[2:]],
        216: [w_copy(1, k) for k in ALL],
    }
    starts = {4: fences[25], 13: fences[47][:1], 25: fences[47][1:], 47: fences[89],
              89: [x_copy(6), x_copy(7), p_copy[5]], 144: fences[216],
              503: [o_copy(bg) for bg in range(5)], 555: [o_copy(5), o_copy(6)],
              571: [o_copy(7, 1), o_copy(7, 2)], 574: [o_copy(7, 0)]}
    x_ready = [f - MARGIN for f in (1, 13, 47, 47, 89, 89, 144, 144)]
    w_ready = [f - MARGIN for f in (4, 25, 47, 89, 216, 216, 216, 216)]
    out_block = (499, 500, 501, 502, 503, 554, 555, None)
    emb_stream = [emb_part(e, 178 + 2 * e) for e in range(9)]
    stat_streams = [x_stats(bg) for bg in range(8)] + [out_stage(i) for i in range(8)]
    for bg in range(8):
        stat_streams[bg][0].release = x_ready[bg]
    in_stream = []
    for idx in range(16):
        in_stream += in_stage(idx, stat_streams[idx][-1])
        if idx == 0:
            for p in in_stream[:80]:
                p.deadline = 0
            in_stream.insert(80, waiting(w_copy(0, 0, 0)))
            w_landed = in_stream[80]
    split, whole = ((0,), (5,), (1, 2), (3, 4)), (JJ_ORDER,)
    w_stream = []
    for k in ALL:
        for jjs in split:
            for n in ALL:
                w_stream += w_stage(0, n, k, (jjs,))
    w_stream[0].after = w_landed
    for n in ALL:
        for k in ALL:
            w_stream += w_stage(1, n, k, whole)
    plan = _plan(stat_streams + [in_stream, w_stream, emb_stream]
                 + [out_stage(i) for i in range(8, 16)])

    running = {}

    def advance(slot):
        pend = []
        for p in plan[slot + 1]:
            if id(p) not in running:
                running[id(p)] = p.emit()
            pend += next(running[id(p)])
        return pend

    def matmuls(lo, hi, zero):
        keeps = [ts[0, i, 0:8, :] == 0.0 for i in range(4)]
        for mm in range(lo, hi):
            s, t = divmod(mm, 36)
            unit, ks, ns, acc = JOBS[s]
            ij = (t % 6) * 6 + JJ_ORDER[t // 6]
            if s == len(JOBS) - 1:
                ij = (1, 2, 3, 4, 0, 5)[t // 6] * 6 + t % 6
            blocks = [[] for _ in ks]
            src = ij if s < 6 or 36 * s <= lo else ij + zero * (s % 4)
            whole = [vw[unit % 2][src, k] for k in ks]
            for r in range(16):
                pend = advance(16 * mm + r)
                w = [lax.slice(v, (8 * r, 0), (8 * r + 8, 128)) for v in whole]
                for i, a in enumerate(pend[-4 * len(ks):]):
                    w[i % len(ks)] = lax.select(
                        keeps[i // len(ks)], w[i % len(ks)], lax.bitcast_convert_type(a, U32))
                for b, v in zip(blocks, w):
                    b.append(v)
            lhs = lax.concatenate(
                [pltpu.bitcast(lax.concatenate(b, 0), BF16) for b in blocks], 1)
            rhs = lax.concatenate([lax.concatenate(
                [pltpu.bitcast(uw[u_slot(unit // 2, n), ij, k], BF16) for k in ks], 1) for n in ns], 0)
            res = lax.dot_general(lhs, rhs, (((1,), (1,)), ((), ())),
                                  preferred_element_type=F32)
            for i, n in enumerate(ns):
                mb = unit % 2 * 4 + n
                v = res[:, 128 * i:128 * (i + 1)]
                ms[mb, ij] = _add(ms[mb, ij], v) if acc else v
        if hi == NMM:
            advance(16 * NMM)

    for cp in p_copy[:5]:
        cp.start()
    for n in range(4):
        x_copy(0, n).start()
    for j in (0, 2, 1):
        w_copy(0, 0, j).start()
    ts[0] = jnp.zeros((6, 16, 128), F32)
    ts[65] = jnp.zeros((6, 16, 128), F32)
    zero = lax.fori_loop(0, 3, lambda i, c: c + i, 0) - 3

    advance(-1)
    for lo, hi in zip((0,) + FENCES, FENCES + (NMM,)):
        for cp in fences.get(lo, ()):
            cp.wait()
        for cp in starts.get(lo, ()):
            cp.start()
        pl.when(zero <= lo)(lambda: matmuls(lo, hi, zero))
    o_copy(7, 3).start()
    for bg in range(7):
        o_copy(bg).wait()
    for n in range(4):
        o_copy(7, n).wait()


@jax.jit
def pallas_standalone__adm_resblock__diffusion_kernel(
        x, t_emb, g1, be1, w1, w_emb, g2, be2, w2):
    B, C, H, W = x.shape
    E = t_emb.shape[1]
    assert (B, C, H, W, E) == (2, 512, 64, 64, 1152)
    xt = x.transpose(0, 2, 3, 1).reshape(B, H // 4, 4, W, C)
    hbm = pl.BlockSpec(memory_space=pl.ANY)
    out = pl.pallas_call(
        _kernel,
        out_shape=jax.ShapeDtypeStruct(xt.shape, x.dtype),
        in_specs=[hbm] * 9,
        out_specs=hbm,
        scratch_shapes=[
            pltpu.VMEM((8, 16, 4, W, 128), BF16),
            pltpu.VMEM((2, 4, 3, 3, 512, 128), BF16),
            pltpu.VMEM((E, C), BF16),
            pltpu.VMEM((B, E), BF16),
            [pltpu.VMEM((C,), BF16)] * 4,
            pltpu.VMEM((5, 36, 4, 128, 128), BF16),
            pltpu.VMEM((36, 4, 256, 128), BF16),
            pltpu.VMEM((36, 4, 256, 128), BF16),
            pltpu.VMEM((8, 36, 256, 128), F32),
            pltpu.VMEM((8, 64, 4, 16, 128), F32),
            pltpu.VMEM((66, 6, 16, 128), F32),
            pltpu.VMEM((B, C), F32),
            pltpu.VMEM((16, 2, 8, 128), F32),
            pltpu.VMEM((16, 2, 8, 128), F32),
            pltpu.SemaphoreType.DMA((12,)),
            pltpu.SemaphoreType.DMA((11,)),
            pltpu.SemaphoreType.DMA((6,)),
            pltpu.SemaphoreType.DMA((12,)),
        ],
        compiler_params=pltpu.CompilerParams(
            vmem_limit_bytes=126 * 2 ** 20, disable_semaphore_checks=True),
        name="resblock",
    )(xt, t_emb, g1, be1, w1.transpose(2, 3, 0, 1), w_emb, g2, be2, w2.transpose(2, 3, 0, 1))
    return out.reshape(B, H, W, C).transpose(0, 3, 1, 2)
```

```python
import jax
import jax.numpy as jnp
import numpy as np
from jax import lax
import jax.experimental.pallas as pl
import jax.experimental.pallas.tpu as pltpu

F32, BF16, U32 = jnp.float32, jnp.bfloat16, jnp.uint32

PA, PB = 1.5, 2.0 / 3.0
NA = 2.0 * PA * PA * (PA * PA - PB * PB)
EPS = 1e-5

JJ_ORDER = (0, 5, 1, 2, 3, 4)
ALL = (0, 1, 2, 3)
JOBS = (
    (0, (0,), ALL, False), (0, (1,), ALL, True), (0, (2,), ALL, True), (0, (3,), ALL, True),
    (1, (0,), ALL, False), (1, (1,), ALL, True),
    (1, (2, 3), (0, 1), True), (1, (2, 3), (2, 3), True),
    (2, ALL, (0,), False), (2, ALL, (1,), False), (2, ALL, (2,), False), (2, ALL, (3,), False),
    (3, ALL, (0,), False), (3, ALL, (1,), False), (3, ALL, (2,), False), (3, ALL, (3,), False),
)
FENCES = (4, 13, 32, 63, 112, 165, 216, 288, 503, 555, 571, 574)
BY_COLUMN = (0, 7)
NMM = 36 * len(JOBS)
MARGIN = 2
LATENCY = 2
STREAM_RATE = 600
STORE_RATE = 139
ALU0 = 49
ALU1 = 47
ALU2 = 45
ALU3 = 42
ALU_RATE = (ALU0,) * 6 + (ALU1,) * 2 + (ALU2,) * 4 + (ALU3,) * 4


def u_slot(c, n):
    return (4 * c + n) % 5


_add, _sub = lax.add, lax.sub


def _mul(x, c):
    return x if abs(c - 1.0) < 1e-12 else lax.mul(x, np.float32(c))


IN_SCALE = (PA, PA * PA, PB, 1.0)
W_SCALE = PA ** 3 / NA ** 2


def _in_tf(d0, d1, d2, d3, d4, d5):
    p = _mul(d2, PB ** 4)
    ea, eb = _sub(d4, p), _sub(d4, d2)
    r0 = _add(_sub(d0, p), eb)
    t = _mul(d3, PA ** 4)
    oa, ob = _mul(_sub(t, d1), PB * PB), _sub(d3, d1)
    r5 = _sub(_sub(d5, t), ob)
    return r0, _add(ea, oa), _sub(ea, oa), _add(eb, ob), _sub(eb, ob), r5


def _out_tf(m0, m1, m2, m3, m4, m5):
    sa, da = _add(m1, m2), _sub(m1, m2)
    sb, db = _add(m3, m4), _sub(m3, m4)
    y0 = _sub(_add(m0, sa), _mul(sb, PA ** 4))
    y1 = _sub(da, _mul(db, PA * PA))
    y2 = _sub(sa, sb)
    y3 = _add(_sub(da, _mul(db, PB * PB)), m5)
    return y0, y1, y2, y3


def _w_tf(g0, g1, g2):
    ea = _add(g0, g2)
    eb, ob = _add(g0, _mul(g2, PB ** 4)), _mul(g1, PB * PB)
    return (_mul(g0, NA), _add(ea, g1), _sub(ea, g1), _add(eb, ob), _sub(eb, ob),
            _mul(g2, NA / PA ** 6))


def _lo(w):
    return lax.bitcast_convert_type(lax.shift_left(w, np.uint32(16)), F32)


def _hi(w):
    return lax.bitcast_convert_type(lax.bitwise_and(w, np.uint32(0xFFFF0000)), F32)


def _cat(a, b):
    return lax.concatenate([a, b], 0)


class _Piece:
    def __init__(self, emit, costs, deadline, release=-1, after=None):
        self.emit, self.costs = emit, np.array(costs, float)
        self.deadline = deadline
        self.release = release
        self.after = after
        self.time, self.gap = None, False


def _plan(streams):
    for st in streams:
        for p in st:
            p.soft = float(p.deadline)
    for _ in range(4):
        for st in streams:
            for i in reversed(range(len(st))):
                p = st[i]
                start = p.soft - p.costs[:, 0].sum() / STREAM_RATE
                if i:
                    st[i - 1].deadline = min(st[i - 1].deadline, p.deadline)
                    st[i - 1].soft = min(st[i - 1].soft, start)
                if p.after is not None:
                    p.after.deadline = min(p.after.deadline, p.deadline)
                    p.after.soft = min(p.after.soft, start - LATENCY)
    pos = [0] * len(streams)
    plan = [[] for _ in range(16 * NMM + 2)]
    cur, credit, rate = None, np.zeros(2), np.zeros(2)

    def pick(mm):
        best = None
        for i, st in enumerate(streams):
            if pos[i] == len(st):
                continue
            p = st[pos[i]]
            urgent = p.deadline <= max(mm, 0) + (left == 0) or mm > NMM
            if not urgent and (mm < 0 or p.release + MARGIN > mm):
                continue
            if p.gap and not urgent and st[pos[i] - 1].time in (None, mm, mm - 1):
                continue
            if p.after is not None and (p.after.time is None or (
                    not urgent and p.after.time + LATENCY > mm)):
                continue
            key = (not urgent, credit[1] <= 0 and p.costs[:, 1].any(), p.soft)
            if best is None or key < best[0]:
                best = key, i
        return best

    def affordable(cost):
        return all(c > 0 or not need for c, need in zip(credit, cost))

    for slot in range(-1, 16 * NMM + 1):
        mm = slot // 16 if slot < 16 * NMM else NMM + 1
        if 0 <= mm < NMM:
            _, ks, ns, acc = JOBS[mm // 36]
            rate = np.array([ALU_RATE[mm // 36] - 2 * len(ns) * (len(ks) - (not acc)),
                             STORE_RATE / 10 - 2 * len(ns)])
            credit = np.minimum(credit + rate, 2 * rate)
        left = min([16 * f - 1 - slot for f in FENCES if 16 * f > slot], default=1000)
        while True:
            best = pick(mm)
            if cur is None:
                if best is None:
                    break
                i = best[1]
                p = streams[i][pos[i]]
                if best[0][0] and not (affordable(p.costs.sum(0)) and all(
                        p.costs.sum(0) <= credit + left * rate)):
                    break
                assert p.release < max(mm, 0) and (mm < p.deadline or mm not in FENCES)
                pos[i] += 1
                cur = [p, 0]
            p, k = cur
            if not affordable(p.costs[k]) and left and p.deadline > max(mm, 0) and (
                    mm <= NMM and (best is None or best[0][0])):
                break
            plan[slot + 1].append(p)
            credit = np.maximum(credit - p.costs[k], -2 * rate)
            cur[1] += 1
            if cur[1] == len(p.costs):
                p.time, cur = mm, None
    assert all(n == len(st) for n, st in zip(pos, streams))
    return plan


def _kernel(x_hbm, t_hbm, g1_hbm, be1_hbm, w1_hbm, we_hbm, g2_hbm, be2_hbm, w2_hbm,
            o_hbm,
            xs, ws, wes, tv, gv, us, v0, v1, ms, hs, ts, emb_s, acc_s, cf,
            xsem, wsem, psem, osem):
    xw = xs.bitcast(U32)
    uw = us.bitcast(U32)
    vs = (v0, v1)
    vw = (v0.bitcast(U32), v1.bitcast(U32))

    def x_copy(bg, part=None):
        rows = slice(None) if part is None else pl.ds(4 * part, 4)
        return pltpu.make_async_copy(
            x_hbm.at[bg // 4, rows, :, :, pl.ds(bg % 4 * 128, 128)], xs.at[bg, rows],
            xsem.at[bg if part is None else 8 + part])

    def w_copy(c, k, j=None):
        cols = slice(None) if j is None else pl.ds(j, 1)
        return pltpu.make_async_copy(
            (w1_hbm, w2_hbm)[c].at[:, cols, :, pl.ds(k * 128, 128)], ws.at[c, k, :, cols],
            wsem.at[4 * c + k if j is None else 8 + j])

    def o_copy(bg, part=None):
        rows = slice(None) if part is None else pl.ds(part, 1)
        return pltpu.make_async_copy(
            xs.at[bg, :, rows], o_hbm.at[bg // 4, :, rows, :, pl.ds(bg % 4 * 128, 128)],
            osem.at[bg if part is None else 8 + part])

    p_copy = [pltpu.make_async_copy(src, dst, psem.at[i]) for i, (src, dst) in enumerate(
        ((g1_hbm, gv[0]), (be1_hbm, gv[1]), (g2_hbm, gv[2]), (be2_hbm, gv[3]),
         (t_hbm, tv), (we_hbm, wes)))]

    def start_rest():
        for cp in fences[13]:
            cp.start()
        yield []

    def waiting(*copies):
        def emit():
            for cp in copies:
                cp.wait()
            yield []
        return _Piece(emit, [(1, 0)], NMM + 1)

    def uses(pred):
        t = [36 * s + 6 * n + ii for s, job in enumerate(JOBS)
             for n, jj in enumerate(JJ_ORDER) for ii in range(6) if pred(job, jj)]
        return min(t), max(t)


    latest = []

    def leash(v):
        return lax.select(ts[0, 0, 0:8, :] == 0.0, v, latest[0]) if latest else v

    def finalize(idx):
        def emit():
            coefficients(idx)
            yield []
        fin = _Piece(emit, [(30, 0)], NMM + 1)
        fin.gap = True
        return fin

    def coefficients(idx):
        g = idx % 4
        s1, s2 = acc_s[idx, 0], acc_s[idx, 1]
        emb = emb_s[pl.ds(idx // 4 - 2, 1), pl.ds(128 * g, 128)] if idx >= 8 else None
        gamma, beta = (r[...].astype(F32).reshape(1, 512)[:, 128 * g:128 * (g + 1)]
                       for r in gv[idx // 8 * 2:idx // 8 * 2 + 2])
        m, q = s1 * (1.0 / 4096.0), s2 * (1.0 / 4096.0)
        if emb is not None:
            m, q = m + emb * 0.125, q + emb * (2.0 * m + emb * 0.125)
        v = _cat(m, q) * (1.0 / 128.0)
        if idx == 0:
            v = jnp.sum(v, axis=1, keepdims=True)
        else:
            parts = []
            for _ in range(4):
                parts.append(v.astype(BF16))
                v = v - parts[-1].astype(F32)
            v = jnp.dot(lax.concatenate(parts, 1), jnp.ones((512, 128), BF16),
                        preferred_element_type=F32)
        mu = jnp.sum(v[:8], axis=0, keepdims=True)
        var = jnp.maximum(jnp.sum(v[8:], axis=0, keepdims=True) - mu * mu, 0.0)
        sc = lax.rsqrt(var + EPS) * gamma * 0.5
        sh = (0.5 * beta) - (mu if emb is None else mu - emb) * sc
        cf[idx, 0] = jnp.broadcast_to(sc, (8, 128))
        cf[idx, 1] = jnp.broadcast_to(sh, (8, 128))

    def x_row(bg, h):
        w = [xw[bg, h // 4, h % 4, pl.ds(k, 8, stride=4), :] for k in range(4)]
        w02, w13 = _cat(w[0], w[2]), _cat(w[1], w[3])
        return [_lo(w02), _hi(w02), _lo(w13), _hi(w13)]

    def x_stats(bg):
        def part(n):
            def emit():
                acc = [acc_s[bg, 0], acc_s[bg, 1]] if n else [None, None]
                for r in range(8 * n, 8 * n + 8):
                    if bg:
                        w = xw[bg, r // 4, r % 4]
                        lo, hi = _lo(w), _hi(w)
                    else:
                        y = x_row(0, r)
                        for j in range(4):
                            hs[7, r, j] = y[j]
                        lo, hi = _cat(y[0], y[1]), _cat(y[2], y[3])
                    a = _add(lo, hi)
                    q = _add(lax.mul(lo, lo), lax.mul(hi, hi))
                    for i, v in enumerate((a, q)):
                        v = _add(v[:16], v[16:])
                        v = _add(v[:8], v[8:])
                        acc[i] = v if acc[i] is None else _add(acc[i], v)
                    if r % 8 == 7:
                        acc_s[bg, 0], acc_s[bg, 1] = acc
                    yield list(acc)
            return _Piece(emit, [(34, 0)] * 8, NMM + 1)

        out = []
        for n in range(8):
            if bg == 0 and n % 2 == 0:
                out.append(waiting(x_copy(0, n // 2)))
            out.append(part(n))
        if bg == 0:
            out += [waiting(*p_copy[:2]), _Piece(start_rest, [(1, 0)], NMM + 1)]
        return out + [finalize(bg)]

    def in_stage(idx, stats):
        unit, g = idx // 4, idx % 4

        def row(h):
            def emit():
                sc, sh = leash(cf[idx, 0]), cf[idx, 1]
                sc, sh = _cat(sc, sc), _cat(sh, sh)
                if 0 < idx < 8:
                    y = x_row(idx, h)
                else:
                    y = [hs[(idx - 8) if idx else 7, h, j] for j in range(4)]
                a = []
                for j, yj in enumerate(y):
                    u = _add(lax.mul(yj, sc), sh)
                    v = _mul(u, IN_SCALE[h % 4] * IN_SCALE[j])
                    a.append(_add(v, lax.mul(v, lax.tanh(u))))
                yield [a[3][8:]]
                sub = lax.broadcasted_iota(jnp.int32, (8, 128), 0)
                pad = jnp.zeros((8, 128), F32)
                left = lax.select(sub == 0, pad, pltpu.roll(a[3][8:], 1, 0))
                right = lax.select(sub == 7, pad, pltpu.roll(a[0][:8], 7, 0))
                r = _in_tf(_cat(left, a[3][:8]), a[0], a[1], a[2], a[3], _cat(a[0][8:], right))
                for jj in range(6):
                    ts[h + 1, jj] = r[jj]
                yield [r[4][:8], r[4][8:]]
            return _Piece(emit, [(47 if idx < 8 else 39, 0), (36, 12)], NMM + 1, after=stats)

        def col(th, jj, deadline, release):
            def emit():
                r = _in_tf(*[ts[4 * th + i, jj] for i in range(6)])
                for ii in range(6):
                    vs[unit % 2][ii * 6 + jj, g, pl.ds(th * 16, 16), :] = r[ii].astype(BF16)
                yield [r[4][:8], r[4][8:]]
            return _Piece(emit, [(38, 6)], deadline, release)

        when = {}
        for jj in JJ_ORDER:
            first = uses(lambda j, q: j[0] == unit and g in j[1] and q == jj)[0]
            prev = -1 if unit < 2 else uses(
                lambda j, q: j[0] == unit - 2 and g in j[1] and q == jj)[1]
            when[jj] = first if first in FENCES else first - MARGIN, prev
        if idx in BY_COLUMN:
            rows = [row(h) for h in range(64)]
            if idx == 7:
                rows[-1].deadline = 200
            return rows + [
                col(th, jj, *when[jj]) for jj in JJ_ORDER for th in range(16)]
        out = [row(h) for h in range(6)]
        if unit == 2:
            out[0].release = 216 - MARGIN
        for th in range(16):
            out += [col(th, jj, *when[jj]) for jj in JJ_ORDER]
            out += [row(h) for h in range(4 * th + 6, min(64, 4 * th + 10))]
        return out

    def out_stage(idx):
        unit, g = idx // 4, idx % 4
        bg = idx % 8
        last = uses(lambda j, q: j[0] == unit and g in j[2])[1]
        mb = idx % 8
        deadline = (208 + 2 * g, NMM)[unit] if unit < 2 else out_block[bg]

        def rows(th, e, z):
            r = pl.ds(th * 16 + e * 8, 8)
            for i in range(6):
                m = [ms[mb, i * 6 + j, r, :] for j in range(6)]
                if unit >= 2:
                    m[1], m[3] = leash(m[1]), leash(m[3])
                z.append(_out_tf(*m))
                yield [z[-1][3]]

        def pixels(z, q):
            y = _out_tf(*[z[i][q] for i in range(6)])
            return [_mul(y[p], PA ** (p + q - 3)) for p in range(4)]

        def hidden(th, e):
            def emit():
                z = []
                yield from rows(th, e, z)
                acc = [acc_s[idx + 8, 0], acc_s[idx + 8, 1]] if th or e else [None, None]
                for q in range(4):
                    y = pixels(z, q)
                    for p in range(4):
                        hs[bg, 4 * th + p, q, pl.ds(e * 8, 8), :] = y[p]
                    sq = [lax.mul(v, v) for v in y]
                    for i, v in enumerate((y, sq)):
                        v = _add(_add(v[0], v[1]), _add(v[2], v[3]))
                        acc[i] = v if acc[i] is None else _add(acc[i], v)
                    if q == 3:
                        acc_s[idx + 8, 0], acc_s[idx + 8, 1] = acc
                    yield list(acc) if q == 3 else acc[1:]
            return _Piece(emit, [(14, 0)] * 6 + [(29, 4.5)] * 4, deadline, last)

        def residual(th, e, p, kq):
            w = xw[bg, th, p, pl.ds(2 * e + kq, 8, stride=4), :]
            return _lo(w), _hi(w)

        def put(th, e, p, kq, lo, hi):
            v = lax.bitcast_convert_type(_cat(lo, hi).astype(BF16).astype(F32), U32)
            v = lax.bitwise_or(lax.shift_right_logical(v[:8], np.uint32(16)), v[8:])
            xw[bg, th, p, pl.ds(2 * e + kq, 8, stride=4), :] = v
            return v

        def closing(phase, th, e):
            r, half = pl.ds(th * 16 + e * 8, 8), pl.ds(e * 8, 8)

            def line(i):
                return _out_tf(*[ms[mb, i * 6 + j, r, :] for j in range(6)])

            def scale(v, p, q, f=1.0):
                return _mul(v, f * PA ** (p + q - 3))

            def emit():
                if phase < 2:
                    z1 = line(2 * phase + 1)
                    yield [z1[3]]
                    z2 = line(2 * phase + 2)
                    yield [z2[3]]
                    sd = [(_add(u, v), _sub(u, v)) for u, v in zip(z1, z2)]
                    for p in range(4):
                        if phase == 0:
                            x = residual(th, e, p, 0) + residual(th, e, p, 1)
                            y = [_add(scale(sd[q][p % 2], p, q), x[q]) for q in range(4)]
                        else:
                            y = [_sub(ts[4 * th + p + 1, q, half, :],
                                      scale(sd[q][p % 2], p, q, PA ** (4 - 2 * p)))
                                 for q in range(4)]
                        if phase == 1 and p in (1, 2):
                            y = [put(th, e, p, kq, *y[2 * kq:2 * kq + 2]) for kq in range(2)]
                        else:
                            for q in range(4):
                                ts[4 * th + p + 1, q, half, :] = y[q]
                        yield y[-1:]
                else:
                    p = 3 * (phase - 2)
                    z = line(5 * (phase - 2))
                    y = [_add(ts[4 * th + p + 1, q, half, :], scale(z[q], p, q))
                         for q in range(4)]
                    yield [put(th, e, p, kq, *y[2 * kq:2 * kq + 2]) for kq in range(2)]

            costs = ([(14, 0)] * 2 + [(14, 4)] * 4, [(14, 0)] * 2 + [(17, 3)] * 4,
                     [(35, 2)], [(35, 2)])[phase]
            return _Piece(emit, costs, (571, 571, 574, NMM + 1)[phase],
                          NMM - 1 - (24, 12, 6, 0)[phase] - (phase > 0))

        def final(th, e):
            def emit():
                z = []
                yield from rows(th, e, z)
                for kq in range(2):
                    y0 = pixels(z, 2 * kq)
                    yield [y0[3]]
                    y1 = pixels(z, 2 * kq + 1)
                    yield [y1[3]]
                    for p in range(4):
                        lo, hi = residual(th, e, p, kq)
                        yield [put(th, e, p, kq, _add(y0[p], lo), _add(y1[p], hi))]
            return _Piece(emit, [(14, 0)] * 6 + ([(18, 0)] * 2 + [(11, 1)] * 4) * 2, deadline, last)

        if unit < 2:
            fin = finalize(idx + 8)
            fin.after = emb_stream[-1]
            fin.deadline = deadline
            return [hidden(th, e) for th in range(16) for e in range(2)] + [fin]
        if idx == 15:
            return [closing(n, th, e) for n in range(4) for th in range(16) for e in range(2)]
        return [final(th, e) for th in range(16) for e in range(2)]

    def w_stage(c, n, k, phases):
        def piece(r, jjs):
            def emit():
                def out(jj, t):
                    u = _w_tf(*t)
                    for ii in range(6):
                        us[u_slot(c, n), ii * 6 + jj, k, pl.ds(r * 16, 16), :] = u[ii].astype(BF16)
                    return [u[i][h:h + 8] for i in ((2, 4) if jj in (0, 5) else (4,))
                            for h in (0, 8)]

                def tap(j):
                    return [ws[c, k if jjs[0] in (0, 5) else k + zero * jjs[0],
                               i, j, pl.ds(128 * n + 16 * r, 16), :].astype(F32)
                            for i in range(3)]

                def scaled(g, f):
                    return [_mul(g[i], W_SCALE * PA ** i * f) for i in range(3)]

                g = {j: tap(j) for j in {(0,): (0,), (5,): (2,)}.get(jjs, (0, 2, 1))}
                if 0 in jjs:
                    yield out(0, scaled(g[0], NA))
                if 5 in jjs:
                    yield out(5, scaled(g[2], NA / PA ** 4))
                if len(jjs) == 2:
                    g = [scaled(g[j], (PA if 1 in jjs else PB) ** j) for j in range(3)]
                    e = [_add(*v) for v in zip(g[0], g[2])]
                    yield out(jjs[0], [_add(*v) for v in zip(e, g[1])])
                    yield out(jjs[1], [_sub(*v) for v in zip(e, g[1])])
                elif len(jjs) == 6:
                    g = [scaled(g[j], PA ** j) for j in range(3)]
                    e = [_add(u, _mul(v, PB ** 4)) for u, v in zip(g[0], g[2])]
                    o = [_mul(v, PB * PB) for v in g[1]]
                    yield out(3, [_add(*v) for v in zip(e, o)])
                    yield out(4, [_sub(*v) for v in zip(e, o)])
                    e = [_add(*v) for v in zip(g[0], g[2])]
                    yield out(1, [_add(*v) for v in zip(e, g[1])])
                    yield out(2, [_sub(*v) for v in zip(e, g[1])])
            return emit

        res = []
        for jjs in phases:
            first = uses(lambda j, q: j[0] // 2 == c and k in j[1] and n in j[2] and q in jjs)[0]
            prev = 288 - MARGIN if c and n else -1
            if (c, k, jjs) != (0, 0, (0,)):
                prev = max(prev, w_ready[4 * c + k])
            costs = {1: [42], 2: [76, 34], 6: [42, 42, 76, 34, 40, 34]}[len(jjs)]
            costs = [(v, 6) for v in costs]
            res += [_Piece(piece(r, jjs), costs,
                           first if first in FENCES else first - (1 if first < 40 else 3), prev) for r in range(8)]
        return res

    def emb_part(e, release):
        def emit():
            t = tv[:, pl.ds(128 * e, 128)].astype(F32)
            t = (t * jax.nn.sigmoid(t)).astype(BF16)
            v = jnp.dot(t, wes[pl.ds(128 * e, 128), :], preferred_element_type=F32)
            emb_s[...] = emb_s[...] + v if e else v
            yield []
        return _Piece(emit, [(20, 4)], release + 5, release)

    fences = {
        4: [w_copy(0, 0, 2), w_copy(0, 0, 1)],
        13: [x_copy(1)],
        32: [w_copy(0, 1), x_copy(2)],
        63: [w_copy(0, 2), x_copy(3), w_copy(0, 3)],
        112: [x_copy(bg) for bg in range(4, 8)] + p_copy[2:],
        216: [w_copy(1, k) for k in ALL],
    }
    starts = {4: fences[32][:1], 13: fences[32][1:] + fences[63][:1],
              32: fences[63][1:] + fences[112][:1], 63: fences[112][1:4] + p_copy[5:],
              112: fences[216],
              503: [o_copy(bg) for bg in range(5)], 555: [o_copy(5), o_copy(6)],
              571: [o_copy(7, 1), o_copy(7, 2)], 574: [o_copy(7, 0)]}
    x_ready = [f - MARGIN for f in (1, 13, 32, 63, 112, 112, 112, 112)]
    w_ready = [f - MARGIN for f in (4, 32, 63, 63, 216, 216, 216, 216)]
    out_block = (499, 500, 501, 502, 503, 554, 555, None)
    emb_stream = [emb_part(e, 116 + 2 * e) for e in range(9)]
    stat_streams = [x_stats(bg) for bg in range(8)] + [out_stage(i) for i in range(8)]
    for bg in range(8):
        stat_streams[bg][0].release = x_ready[bg]
    in_stream = []
    for idx in range(16):
        in_stream += in_stage(idx, stat_streams[idx][-1])
        if idx == 0:
            for p in in_stream[:80]:
                p.deadline = 0
            in_stream.insert(80, waiting(w_copy(0, 0, 0)))
            w_landed = in_stream[80]
    split, whole = ((0,), (5,), (1, 2), (3, 4)), (JJ_ORDER,)
    w_stream = []
    for k in ALL:
        for jjs in split:
            for n in ALL:
                w_stream += w_stage(0, n, k, (jjs,))
    w_stream[0].after = w_landed
    for n in ALL:
        for k in ALL:
            w_stream += w_stage(1, n, k, whole)
    plan = _plan(stat_streams + [in_stream, w_stream, emb_stream]
                 + [out_stage(i) for i in range(8, 16)])

    running = {}

    def advance(slot):
        pend = []
        for p in plan[slot + 1]:
            if id(p) not in running:
                running[id(p)] = p.emit()
            pend += next(running[id(p)])
        return pend

    def matmuls(lo, hi, zero):
        keeps = [ts[0, i, 0:8, :] == 0.0 for i in range(4)]
        for mm in range(lo, hi):
            s, t = divmod(mm, 36)
            unit, ks, ns, acc = JOBS[s]
            ij = (t % 6) * 6 + JJ_ORDER[t // 6]
            if s == len(JOBS) - 1:
                ij = (1, 2, 3, 4, 0, 5)[t // 6] * 6 + t % 6
            blocks = [[] for _ in ks]
            src = ij if s < 6 or 36 * s <= lo else ij + zero * (s % 4)
            whole = [vw[unit % 2][src, k] for k in ks]
            for r in range(16):
                pend = advance(16 * mm + r)
                w = [lax.slice(v, (8 * r, 0), (8 * r + 8, 128)) for v in whole]
                for i, a in enumerate(pend[-4 * len(ks):]):
                    w[i % len(ks)] = lax.select(
                        keeps[i // len(ks)], w[i % len(ks)], lax.bitcast_convert_type(a, U32))
                for b, v in zip(blocks, w):
                    b.append(v)
            lhs = lax.concatenate(
                [pltpu.bitcast(lax.concatenate(b, 0), BF16) for b in blocks], 1)
            rhs = lax.concatenate([lax.concatenate(
                [pltpu.bitcast(uw[u_slot(unit // 2, n), ij, k], BF16) for k in ks], 1) for n in ns], 0)
            res = lax.dot_general(lhs, rhs, (((1,), (1,)), ((), ())),
                                  preferred_element_type=F32)
            for i, n in enumerate(ns):
                mb = unit % 2 * 4 + n
                v = res[:, 128 * i:128 * (i + 1)]
                ms[mb, ij] = _add(ms[mb, ij], v) if acc else v
            latest[:] = [v[:8]] if mm + 1 < hi else []
        if hi == NMM:
            advance(16 * NMM)

    for cp in p_copy[:5]:
        cp.start()
    for n in range(4):
        x_copy(0, n).start()
    for j in (0, 2, 1):
        w_copy(0, 0, j).start()
    ts[0] = jnp.zeros((6, 16, 128), F32)
    ts[65] = jnp.zeros((6, 16, 128), F32)
    zero = lax.fori_loop(0, 3, lambda i, c: c + i, 0) - 3

    advance(-1)
    for lo, hi in zip((0,) + FENCES, FENCES + (NMM,)):
        for cp in fences.get(lo, ()):
            cp.wait()
        for cp in starts.get(lo, ()):
            cp.start()
        pl.when(zero <= lo)(lambda: matmuls(lo, hi, zero))
    o_copy(7, 3).start()
    for bg in range(7):
        o_copy(bg).wait()
    for n in range(4):
        o_copy(7, n).wait()


@jax.jit
def pallas_standalone__adm_resblock__diffusion_kernel(
        x, t_emb, g1, be1, w1, w_emb, g2, be2, w2):
    B, C, H, W = x.shape
    E = t_emb.shape[1]
    assert (B, C, H, W, E) == (2, 512, 64, 64, 1152)
    xt = x.transpose(0, 2, 3, 1).reshape(B, H // 4, 4, W, C)
    hbm = pl.BlockSpec(memory_space=pl.ANY)
    out = pl.pallas_call(
        _kernel,
        out_shape=jax.ShapeDtypeStruct(xt.shape, x.dtype),
        in_specs=[hbm] * 9,
        out_specs=hbm,
        scratch_shapes=[
            pltpu.VMEM((8, 16, 4, W, 128), BF16),
            pltpu.VMEM((2, 4, 3, 3, 512, 128), BF16),
            pltpu.VMEM((E, C), BF16),
            pltpu.VMEM((B, E), BF16),
            [pltpu.VMEM((C,), BF16)] * 4,
            pltpu.VMEM((5, 36, 4, 128, 128), BF16),
            pltpu.VMEM((36, 4, 256, 128), BF16),
            pltpu.VMEM((36, 4, 256, 128), BF16),
            pltpu.VMEM((8, 36, 256, 128), F32),
            pltpu.VMEM((8, 64, 4, 16, 128), F32),
            pltpu.VMEM((66, 6, 16, 128), F32),
            pltpu.VMEM((B, C), F32),
            pltpu.VMEM((16, 2, 8, 128), F32),
            pltpu.VMEM((16, 2, 8, 128), F32),
            pltpu.SemaphoreType.DMA((12,)),
            pltpu.SemaphoreType.DMA((11,)),
            pltpu.SemaphoreType.DMA((6,)),
            pltpu.SemaphoreType.DMA((12,)),
        ],
        compiler_params=pltpu.CompilerParams(
            vmem_limit_bytes=126 * 2 ** 20, disable_semaphore_checks=True),
        name="resblock",
    )(xt, t_emb, g1, be1, w1.transpose(2, 3, 0, 1), w_emb, g2, be2, w2.transpose(2, 3, 0, 1))
    return out.reshape(B, H, W, C).transpose(0, 3, 1, 2)
```

```python
import jax
import jax.numpy as jnp
import numpy as np
from jax import lax
import jax.experimental.pallas as pl
import jax.experimental.pallas.tpu as pltpu

F32, BF16, U32 = jnp.float32, jnp.bfloat16, jnp.uint32
EPS = 1e-5

PA, PB = 1.5, 2.0 / 3.0
NA = 2.0 * PA * PA * (PA * PA - PB * PB)
IN_SCALE = (PA, PA * PA, PB, 1.0)
W_SCALE = PA ** 3 / NA ** 2

_add, _sub = lax.add, lax.sub


def _mul(x, c):
    return x if abs(c - 1.0) < 1e-12 else lax.mul(x, np.float32(c))


def _out_scale(p, q):
    return PA ** (p + q - 3)


def _in_tf(d0, d1, d2, d3, d4, d5):
    p = _mul(d2, PB ** 4)
    ea, eb = _sub(d4, p), _sub(d4, d2)
    r0 = _add(_sub(d0, p), eb)
    t = _mul(d3, PA ** 4)
    oa, ob = _mul(_sub(t, d1), PB * PB), _sub(d3, d1)
    r5 = _sub(_sub(d5, t), ob)
    return r0, _add(ea, oa), _sub(ea, oa), _add(eb, ob), _sub(eb, ob), r5


def _out_tf(m0, m1, m2, m3, m4, m5):
    sa, da = _add(m1, m2), _sub(m1, m2)
    sb, db = _add(m3, m4), _sub(m3, m4)
    y0 = _sub(_add(m0, sa), _mul(sb, PA ** 4))
    y1 = _sub(da, _mul(db, PA * PA))
    y2 = _sub(sa, sb)
    y3 = _add(_sub(da, _mul(db, PB * PB)), m5)
    return y0, y1, y2, y3


def _w_tf(g0, g1, g2):
    ea = _add(g0, g2)
    eb, ob = _add(g0, _mul(g2, PB ** 4)), _mul(g1, PB * PB)
    return (_mul(g0, NA), _add(ea, g1), _sub(ea, g1), _add(eb, ob), _sub(eb, ob),
            _mul(g2, NA / PA ** 6))


def _lo(w):
    return lax.bitcast_convert_type(lax.shift_left(w, np.uint32(16)), F32)


def _hi(w):
    return lax.bitcast_convert_type(lax.bitwise_and(w, np.uint32(0xFFFF0000)), F32)


def _cat(a, b):
    return lax.concatenate([a, b], 0)


ALL = (0, 1, 2, 3)
JOBS = (
    (0, (0,), ALL, False), (0, (1,), ALL, True), (0, (2,), ALL, True), (0, (3,), ALL, True),
    (1, (0,), ALL, False), (1, (1,), ALL, True),
    (1, (2, 3), (0, 1), True), (1, (2, 3), (2, 3), True),
    (2, ALL, (0,), False), (2, ALL, (1,), False), (2, ALL, (2,), False), (2, ALL, (3,), False),
    (3, ALL, (0,), False), (3, ALL, (1,), False), (3, ALL, (2,), False), (3, ALL, (3,), False),
)
NMM = 36 * len(JOBS)
SLOTS = 16
COL_ORDER = (0, 5, 1, 2, 3, 4)
LAST_ROW_ORDER = (1, 2, 3, 4, 0, 5)
FENCES = (4, 13, 32, 63, 112, 165, 216, 288, 503, 555, 571, 574)
MARGIN = 2
STREAM_RATE = 600
ALU_RATE = (47,) * 3 + (49,) * 3 + (47,) * 2 + (45,) * 4 + (42,) * 4
STORE_RATE = 13.9


class _Piece:
    def __init__(self, emit, costs, deadline=NMM + 1, release=-1, after=None, gap=False):
        self.emit, self.costs = emit, np.array(costs, float)
        self.deadline = deadline
        self.release = release
        self.after = after
        self.gap = gap
        self.start = self.time = self.steps = None


def _plan(streams):
    for st in streams:
        for p in st:
            p.soft = float(p.deadline)
    for _ in range(4):
        for st in streams:
            for i in reversed(range(len(st))):
                p = st[i]
                start = p.soft - p.costs[:, 0].sum() / STREAM_RATE
                if i:
                    st[i - 1].deadline = min(st[i - 1].deadline, p.deadline)
                    st[i - 1].soft = min(st[i - 1].soft, start)
                if p.after is not None:
                    p.after.deadline = min(p.after.deadline, p.deadline)
                    p.after.soft = min(p.after.soft, start - MARGIN)
    pos = [0] * len(streams)
    plan = [[] for _ in range(SLOTS * NMM + 2)]
    cur, credit, rate = None, np.zeros(2), np.zeros(2)

    def pick(mm, left):
        best = None
        for i, st in enumerate(streams):
            if pos[i] == len(st):
                continue
            p = st[pos[i]]
            urgent = p.deadline <= max(mm, 0) + (left == 0) or mm > NMM
            if not urgent and (mm < 0 or p.release + MARGIN > mm):
                continue
            if p.gap and not urgent and st[pos[i] - 1].time in (None, mm, mm - 1):
                continue
            if p.after is not None and (p.after.time is None or (
                    not urgent and p.after.time + MARGIN > mm)):
                continue
            key = (not urgent, credit[1] <= 0 and p.costs[:, 1].any(), p.soft)
            if best is None or key < best[0]:
                best = key, i
        return best

    def affordable(cost):
        return all(c > 0 or not need for c, need in zip(credit, cost))

    for slot in range(-1, SLOTS * NMM + 1):
        mm = slot // SLOTS if slot < SLOTS * NMM else NMM + 1
        if 0 <= mm < NMM:
            _, ks, ns, acc = JOBS[mm // 36]
            rate = np.array([ALU_RATE[mm // 36] - 2 * len(ns) * (len(ks) - (not acc)),
                             STORE_RATE - 2 * len(ns)])
            credit = np.minimum(credit + rate, 2 * rate)
        left = min([SLOTS * f - 1 - slot for f in FENCES if SLOTS * f > slot], default=1000)
        while True:
            best = pick(mm, left)
            if cur is None:
                if best is None:
                    break
                i = best[1]
                p = streams[i][pos[i]]
                if best[0][0] and not (affordable(p.costs.sum(0)) and all(
                        p.costs.sum(0) <= credit + left * rate)):
                    break
                assert p.release < max(mm, 0)
                assert mm < p.deadline or p.deadline not in FENCES
                pos[i] += 1
                p.start, cur = mm, [p, 0]
            p, k = cur
            if not affordable(p.costs[k]) and left and p.deadline > max(mm, 0) and (
                    mm <= NMM and (best is None or best[0][0])):
                break
            plan[slot + 1].append(p)
            credit = np.maximum(credit - p.costs[k], -2 * rate)
            cur[1] += 1
            if cur[1] == len(p.costs):
                p.time, cur = mm, None
    assert all(n == len(st) for n, st in zip(pos, streams))
    return plan


def _uses(pred):
    t = [36 * s + 6 * n + i for s, job in enumerate(JOBS)
         for n, jj in enumerate(COL_ORDER) for i in range(6) if pred(job, jj)]
    return min(t), max(t)


def _u_slot(conv, n):
    return (4 * conv + n) % 5


def _kernel(x_hbm, t_hbm, g1_hbm, be1_hbm, w1_hbm, we_hbm, g2_hbm, be2_hbm, w2_hbm, o_hbm,
            xs, ws, wes, tv, gv, us, v0, v1, ms, hs, ts, emb_s, acc_s, cf,
            xsem, wsem, psem, osem):
    xw, uw = xs.bitcast(U32), us.bitcast(U32)
    vs, vw = (v0, v1), (v0.bitcast(U32), v1.bitcast(U32))

    def x_copy(bg, part=None):
        rows = slice(None) if part is None else pl.ds(4 * part, 4)
        return pltpu.make_async_copy(
            x_hbm.at[bg // 4, rows, :, :, pl.ds(bg % 4 * 128, 128)], xs.at[bg, rows],
            xsem.at[bg if part is None else 8 + part])

    def w_copy(conv, k, j=None):
        cols = slice(None) if j is None else pl.ds(j, 1)
        return pltpu.make_async_copy(
            (w1_hbm, w2_hbm)[conv].at[:, cols, :, pl.ds(k * 128, 128)], ws.at[conv, k, :, cols],
            wsem.at[4 * conv + k if j is None else 8 + j])

    def o_copy(bg, part=None):
        rows = slice(None) if part is None else pl.ds(part, 1)
        return pltpu.make_async_copy(
            xs.at[bg, :, rows], o_hbm.at[bg // 4, :, rows, :, pl.ds(bg % 4 * 128, 128)],
            osem.at[bg if part is None else 8 + part])

    p_copy = [pltpu.make_async_copy(src, dst, psem.at[i]) for i, (src, dst) in enumerate(
        ((g1_hbm, gv[0]), (be1_hbm, gv[1]), (g2_hbm, gv[2]), (be2_hbm, gv[3]),
         (t_hbm, tv), (we_hbm, wes)))]

    waits = {
        4: [w_copy(0, 0, 2), w_copy(0, 0, 1)],
        13: [x_copy(1)],
        32: [w_copy(0, 1), x_copy(2)],
        63: [w_copy(0, 2), x_copy(3), w_copy(0, 3)],
        112: [x_copy(bg) for bg in range(4, 8)] + p_copy[2:],
        216: [w_copy(1, k) for k in ALL],
    }
    starts = {
        4: waits[32][:1],
        13: waits[32][1:] + waits[63][:1],
        32: waits[63][1:] + waits[112][:1],
        63: waits[112][1:],
        112: waits[216],
        503: [o_copy(bg) for bg in range(5)],
        555: [o_copy(5), o_copy(6)],
        571: [o_copy(7, 1), o_copy(7, 2)],
        574: [o_copy(7, 0)],
    }
    x_landed = (0, 13, 32, 63, 112, 112, 112, 112)
    w_landed = (4, 32, 63, 63, 216, 216, 216, 216)
    out_due = (499, 500, 501, 502, 503, 554, 555)

    def dma_piece(wait=(), start=()):
        def emit():
            for cp in wait:
                cp.wait()
            for cp in start:
                cp.start()
            yield []
        return _Piece(emit, [(1, 0)])

    keep, latest = [], []

    def leash(v):
        return lax.select(keep[0], v, latest[0]) if latest else v

    def coefficients(idx):
        def emit():
            g = idx % 4
            gamma, beta = (r[...].astype(F32).reshape(1, 512)[:, 128 * g:128 * (g + 1)]
                           for r in gv[idx // 8 * 2:idx // 8 * 2 + 2])
            m, q = acc_s[idx, 0] * (1.0 / 4096.0), acc_s[idx, 1] * (1.0 / 4096.0)
            if idx >= 8:
                emb = emb_s[pl.ds(idx // 4 - 2, 1), pl.ds(128 * g, 128)]
                m, q = m + emb * 0.125, q + emb * (2.0 * m + emb * 0.125)
            v = _cat(m, q) * (1.0 / 128.0)
            if idx == 0 or idx >= 8:
                v = jnp.sum(_cat(leash(v[:8]), leash(v[8:])), axis=1, keepdims=True)
            else:
                parts = []
                for _ in range(4):
                    parts.append(v.astype(BF16))
                    v = v - parts[-1].astype(F32)
                v = jnp.dot(lax.concatenate(parts, 1), jnp.ones((512, 128), BF16),
                            preferred_element_type=F32)
            mu = jnp.sum(v[:8], axis=0, keepdims=True)
            var = jnp.maximum(jnp.sum(v[8:], axis=0, keepdims=True) - mu * mu, 0.0)
            scale = lax.rsqrt(var + EPS) * gamma * 0.5
            shift = 0.5 * beta - (mu - emb if idx >= 8 else mu) * scale
            cf[idx, 0] = jnp.broadcast_to(scale, (8, 128))
            cf[idx, 1] = jnp.broadcast_to(shift, (8, 128))
            yield []
        return _Piece(emit, [(30, 0)], gap=True)

    def x_row(bg, h):
        w = [xw[bg, h // 4, h % 4, pl.ds(k, 8, stride=4), :] for k in range(4)]
        w02, w13 = _cat(w[0], w[2]), _cat(w[1], w[3])
        return [_lo(w02), _hi(w02), _lo(w13), _hi(w13)]

    def x_stats(bg):
        def part(n):
            def emit():
                acc = [acc_s[bg, 0], acc_s[bg, 1]] if n else [None, None]
                for h in range(8 * n, 8 * n + 8):
                    if bg:
                        w = xw[bg, h // 4, h % 4]
                        lo, hi = _lo(w), _hi(w)
                    else:
                        y = x_row(0, h)
                        for j in range(4):
                            hs[7, h, j] = y[j]
                        lo, hi = _cat(y[0], y[1]), _cat(y[2], y[3])
                    for i, v in enumerate((_add(lo, hi),
                                           _add(lax.mul(lo, lo), lax.mul(hi, hi)))):
                        v = _add(v[:16], v[16:])
                        v = _add(v[:8], v[8:])
                        acc[i] = v if acc[i] is None else _add(acc[i], v)
                    if h % 8 == 7:
                        acc_s[bg, 0], acc_s[bg, 1] = acc
                    yield list(acc)
            return _Piece(emit, [(34, 0)] * 8)

        out = []
        for n in range(8):
            if bg == 0 and n % 2 == 0:
                out.append(dma_piece([x_copy(0, n // 2)]))
            out.append(part(n))
        if bg == 0:
            out.append(dma_piece(p_copy[:2], waits[13]))
        else:
            out[0].release = x_landed[bg] - MARGIN
        return out + [coefficients(bg)]

    def in_stage(idx, stats):
        unit, g = idx // 4, idx % 4

        def row(h):
            def emit():
                scale, shift = leash(cf[idx, 0]), cf[idx, 1]
                scale, shift = _cat(scale, scale), _cat(shift, shift)
                if 0 < idx < 8:
                    y = x_row(idx, h)
                else:
                    y = [hs[(idx - 8) if idx else 7, h, j] for j in range(4)]
                a = []
                for j in range(4):
                    u = _add(lax.mul(y[j], scale), shift)
                    v = _mul(u, IN_SCALE[h % 4] * IN_SCALE[j])
                    a.append(_add(v, lax.mul(v, lax.tanh(u))))
                yield [a[3][8:]]
                sub = lax.broadcasted_iota(jnp.int32, (8, 128), 0)
                pad = jnp.zeros((8, 128), F32)
                left = lax.select(sub == 0, pad, pltpu.roll(a[3][8:], 1, 0))
                right = lax.select(sub == 7, pad, pltpu.roll(a[0][:8], 7, 0))
                r = _in_tf(_cat(left, a[3][:8]), a[0], a[1], a[2], a[3], _cat(a[0][8:], right))
                for jj in range(6):
                    ts[h + 1, jj] = r[jj]
                yield [r[4][:8], r[4][8:]]
            return _Piece(emit, [(47 if idx < 8 else 39, 0), (36, 12)], after=stats)

        def col(th, jj):
            def emit():
                r = _in_tf(*[ts[4 * th + i, jj] for i in range(6)])
                for ii in range(6):
                    vs[unit % 2][ii * 6 + jj, g, pl.ds(th * 16, 16), :] = r[ii].astype(BF16)
                yield [r[4][:8], r[4][8:]]
            return _Piece(emit, [(38, 6)], *window[jj])

        window = {}
        for jj in COL_ORDER:
            first = _uses(lambda j, q: j[0] == unit and g in j[1] and q == jj)[0]
            freed = -1 if unit < 2 else _uses(
                lambda j, q: j[0] == unit - 2 and g in j[1] and q == jj)[1]
            window[jj] = first if first in FENCES else first - MARGIN, freed
        if idx in (0, 7):
            rows = [row(h) for h in range(64)]
            if idx == 7:
                rows[-1].deadline = 200
            return rows + [col(th, jj) for jj in COL_ORDER for th in range(16)]
        out = [row(h) for h in range(6)]
        if unit == 2:
            out[0].release = 216 - MARGIN
        for th in range(16):
            out += [col(th, jj) for jj in COL_ORDER]
            out += [row(h) for h in range(4 * th + 6, min(64, 4 * th + 10))]
        return out

    def out_stage(idx):
        unit, g, bg = idx // 4, idx % 4, idx % 8
        last = _uses(lambda j, q: j[0] == unit and g in j[2])[1]

        def load(th, e, i):
            return [ms[bg, i * 6 + j, pl.ds(th * 16 + e * 8, 8), :] for j in range(6)]

        def along_w(th, e, z):
            for i in range(6):
                m = load(th, e, i)
                if unit >= 2:
                    m[1], m[3] = leash(m[1]), leash(m[3])
                z.append(_out_tf(*m))
                yield [z[-1][3]]

        def along_h(z, q):
            y = _out_tf(*[z[i][q] for i in range(6)])
            return [_mul(y[p], _out_scale(p, q)) for p in range(4)]

        def hidden(th, e):
            def emit():
                z = []
                yield from along_w(th, e, z)
                acc = [acc_s[idx + 8, 0], acc_s[idx + 8, 1]] if th or e else [None, None]
                for q in range(4):
                    y = along_h(z, q)
                    for p in range(4):
                        hs[bg, 4 * th + p, q, pl.ds(e * 8, 8), :] = y[p]
                    for i, v in enumerate((y, [lax.mul(v, v) for v in y])):
                        v = _add(_add(v[0], v[1]), _add(v[2], v[3]))
                        acc[i] = v if acc[i] is None else _add(acc[i], v)
                    if q == 3:
                        acc_s[idx + 8, 0], acc_s[idx + 8, 1] = acc
                    yield list(acc) if q == 3 else acc[1:]
            return _Piece(emit, [(14, 0)] * 6 + [(29, 4.5)] * 4, release=last)

        def residual(th, e, p, kq):
            w = xw[bg, th, p, pl.ds(2 * e + kq, 8, stride=4), :]
            return _lo(w), _hi(w)

        def put(th, e, p, kq, lo, hi):
            v = lax.bitcast_convert_type(_cat(lo, hi).astype(BF16).astype(F32), U32)
            v = lax.bitwise_or(lax.shift_right_logical(v[:8], np.uint32(16)), v[8:])
            xw[bg, th, p, pl.ds(2 * e + kq, 8, stride=4), :] = v
            return v

        def final(th, e):
            def emit():
                z = []
                yield from along_w(th, e, z)
                for kq in range(2):
                    y0 = along_h(z, 2 * kq)
                    yield [y0[3]]
                    y1 = along_h(z, 2 * kq + 1)
                    yield [y1[3]]
                    for p in range(4):
                        lo, hi = residual(th, e, p, kq)
                        yield [put(th, e, p, kq, _add(y0[p], lo), _add(y1[p], hi))]
            return _Piece(emit, [(14, 0)] * 6 + ([(18, 0)] * 2 + [(11, 1)] * 4) * 2,
                          out_due[bg], last)

        def closing(phase, th, e):
            half = pl.ds(e * 8, 8)

            def emit():
                if phase < 2:
                    z1 = _out_tf(*load(th, e, 2 * phase + 1))
                    yield [z1[3]]
                    z2 = _out_tf(*load(th, e, 2 * phase + 2))
                    yield [z2[3]]
                    sd = [(_add(u, v), _sub(u, v)) for u, v in zip(z1, z2)]
                    for p in range(4):
                        if phase == 0:
                            x = residual(th, e, p, 0) + residual(th, e, p, 1)
                            y = [_add(_mul(sd[q][p % 2], _out_scale(p, q)), x[q])
                                 for q in range(4)]
                        else:
                            y = [_sub(ts[4 * th + p + 1, q, half, :],
                                      _mul(sd[q][p % 2], PA ** (4 - 2 * p) * _out_scale(p, q)))
                                 for q in range(4)]
                        if phase == 1 and p in (1, 2):
                            y = [put(th, e, p, kq, *y[2 * kq:2 * kq + 2]) for kq in range(2)]
                        else:
                            for q in range(4):
                                ts[4 * th + p + 1, q, half, :] = y[q]
                        yield y[-1:]
                else:
                    p = 3 * (phase - 2)
                    z = _out_tf(*load(th, e, 5 * (phase - 2)))
                    y = [_add(ts[4 * th + p + 1, q, half, :], _mul(z[q], _out_scale(p, q)))
                         for q in range(4)]
                    yield [put(th, e, p, kq, *y[2 * kq:2 * kq + 2]) for kq in range(2)]

            costs = ([(14, 0)] * 2 + [(14, 4)] * 4, [(14, 0)] * 2 + [(17, 3)] * 4,
                     [(35, 2)], [(35, 2)])[phase]
            return _Piece(emit, costs, (571, 571, 574, NMM + 1)[phase],
                          NMM - (25, 14, 8, 2)[phase])

        tiles = [(th, e) for th in range(16) for e in range(2)]
        if unit < 2:
            fin = coefficients(idx + 8)
            fin.after, fin.deadline = emb_stream[-1], (208 + 2 * g, NMM)[unit]
            return [hidden(*t) for t in tiles] + [fin]
        if idx == 15:
            return [closing(n, *t) for n in range(4) for t in tiles]
        return [final(*t) for t in tiles]

    def w_stage(conv, n, k, jjs):
        def piece(r):
            def tap(j):
                return [ws[conv, k if jjs[0] in (0, 5) else k + zero * jjs[0], i, j,
                           pl.ds(128 * n + 16 * r, 16), :].astype(F32) for i in range(3)]

            def scaled(g, f):
                return [_mul(g[i], W_SCALE * PA ** i * f) for i in range(3)]

            def out(jj, t):
                u = _w_tf(*t)
                for ii in range(6):
                    us[_u_slot(conv, n), ii * 6 + jj, k, pl.ds(r * 16, 16), :] = (
                        u[ii].astype(BF16))
                return [u[i][h:h + 8] for i in ((2, 4) if jj in (0, 5) else (4,))
                        for h in (0, 8)]

            def emit():
                g = {j: tap(j) for j in {(0,): (0,), (5,): (2,)}.get(jjs, (0, 2, 1))}
                if 0 in jjs:
                    yield out(0, scaled(g[0], NA))
                if 5 in jjs:
                    yield out(5, scaled(g[2], NA / PA ** 4))
                if len(jjs) == 2:
                    g = [scaled(g[j], (PA if 1 in jjs else PB) ** j) for j in range(3)]
                    e = [_add(*v) for v in zip(g[0], g[2])]
                    yield out(jjs[0], [_add(*v) for v in zip(e, g[1])])
                    yield out(jjs[1], [_sub(*v) for v in zip(e, g[1])])
                elif len(jjs) == 6:
                    g = [scaled(g[j], PA ** j) for j in range(3)]
                    e = [_add(u, _mul(v, PB ** 4)) for u, v in zip(g[0], g[2])]
                    o = [_mul(v, PB * PB) for v in g[1]]
                    yield out(3, [_add(*v) for v in zip(e, o)])
                    yield out(4, [_sub(*v) for v in zip(e, o)])
                    e = [_add(*v) for v in zip(g[0], g[2])]
                    yield out(1, [_add(*v) for v in zip(e, g[1])])
                    yield out(2, [_sub(*v) for v in zip(e, g[1])])
            return emit

        first = _uses(lambda j, q: j[0] // 2 == conv and k in j[1] and n in j[2] and q in jjs)[0]
        deadline = first if first in FENCES else first - (1 if first < 40 else 3)
        release = -1
        if (conv, k, jjs) != (0, 0, (0,)):
            release = max(w_landed[4 * conv + k], 288 if conv and n else 0) - MARGIN
        costs = {1: [42], 2: [76, 34], 6: [42, 42, 76, 34, 40, 34]}[len(jjs)]
        return [_Piece(piece(r), [(v, 6) for v in costs], deadline, release) for r in range(8)]

    def emb_part(e):
        def emit():
            t = tv[:, pl.ds(128 * e, 128)].astype(F32)
            t = (t * jax.nn.sigmoid(t)).astype(BF16)
            v = jnp.dot(t, wes[pl.ds(128 * e, 128), :], preferred_element_type=F32)
            emb_s[...] = emb_s[...] + v if e else v
            yield []
        return _Piece(emit, [(20, 4)], 133 + 3 * e, 128 + 3 * e)

    emb_stream = [emb_part(e) for e in range(9)]
    stat_streams = [x_stats(bg) for bg in range(8)] + [out_stage(i) for i in range(8)]
    in_stream = []
    for idx in range(16):
        in_stream += in_stage(idx, stat_streams[idx][-1])
    in_stream.insert(80, dma_piece([w_copy(0, 0, 0)]))
    w_stream = []
    for k in ALL:
        for jjs in ((0,), (5,), (1, 2), (3, 4)):
            for n in ALL:
                w_stream += w_stage(0, n, k, jjs)
    w_stream[0].after = in_stream[80]
    for n in ALL:
        for k in ALL:
            w_stream += w_stage(1, n, k, COL_ORDER)
    plan = _plan(stat_streams + [in_stream, w_stream, emb_stream]
                 + [out_stage(i) for i in range(8, 16)])
    for p in w_stream + emb_stream + [st[0] for st in stat_streams[1:8]]:
        assert p.release < 0 or p.start >= p.release + MARGIN

    def advance(slot):
        anchors = []
        for p in plan[slot + 1]:
            if p.steps is None:
                p.steps = p.emit()
            anchors += next(p.steps)
        return anchors

    def matmuls(lo, hi):
        keep[:] = [ts[0, i, 0:8, :] == 0.0 for i in range(4)]
        for mm in range(lo, hi):
            s, t = divmod(mm, 36)
            unit, ks, ns, acc = JOBS[s]
            ij = (t % 6) * 6 + COL_ORDER[t // 6]
            if s == len(JOBS) - 1:
                ij = LAST_ROW_ORDER[t // 6] * 6 + t % 6
            src = ij if s < 6 or 36 * s <= lo else ij + zero * (s % 4)
            whole = [vw[unit % 2][src, k] for k in ks]
            blocks = [[] for _ in ks]
            for r in range(SLOTS):
                w = [lax.slice(v, (8 * r, 0), (8 * r + 8, 128)) for v in whole]
                for i, a in enumerate(advance(SLOTS * mm + r)[-4 * len(ks):]):
                    w[i % len(ks)] = lax.select(
                        keep[i // len(ks)], w[i % len(ks)], lax.bitcast_convert_type(a, U32))
                for b, v in zip(blocks, w):
                    b.append(v)
            lhs = lax.concatenate(
                [pltpu.bitcast(lax.concatenate(b, 0), BF16) for b in blocks], 1)
            rhs = lax.concatenate([lax.concatenate(
                [pltpu.bitcast(uw[_u_slot(unit // 2, n), ij, k], BF16) for k in ks], 1)
                for n in ns], 0)
            res = lax.dot_general(lhs, rhs, (((1,), (1,)), ((), ())),
                                  preferred_element_type=F32)
            for i, n in enumerate(ns):
                bg = unit % 2 * 4 + n
                v = res[:, 128 * i:128 * (i + 1)]
                ms[bg, ij] = _add(ms[bg, ij], v) if acc else v
            latest[:] = [v[:8]] if mm + 1 < hi else []
        if hi == NMM:
            advance(SLOTS * NMM)

    for cp in p_copy[:2] + [x_copy(0, n) for n in range(4)] + [
            w_copy(0, 0, j) for j in (0, 2, 1)]:
        cp.start()
    ts[0] = jnp.zeros((6, 16, 128), F32)
    ts[65] = jnp.zeros((6, 16, 128), F32)
    zero = lax.fori_loop(0, 3, lambda i, c: c + i, 0) - 3

    advance(-1)
    for lo, hi in zip((0,) + FENCES, FENCES + (NMM,)):
        for cp in waits.get(lo, ()):
            cp.wait()
        for cp in starts.get(lo, ()):
            cp.start()
        pl.when(zero <= lo)(lambda: matmuls(lo, hi))
    o_copy(7, 3).start()
    for cp in [o_copy(bg) for bg in range(7)] + [o_copy(7, n) for n in range(4)]:
        cp.wait()


@jax.jit
def pallas_standalone__adm_resblock__diffusion_kernel(
        x, t_emb, g1, be1, w1, w_emb, g2, be2, w2):
    B, C, H, W = x.shape
    E = t_emb.shape[1]
    assert (B, C, H, W, E) == (2, 512, 64, 64, 1152)
    xt = x.transpose(0, 2, 3, 1).reshape(B, H // 4, 4, W, C)
    hbm = pl.BlockSpec(memory_space=pl.ANY)
    out = pl.pallas_call(
        _kernel,
        out_shape=jax.ShapeDtypeStruct(xt.shape, x.dtype),
        in_specs=[hbm] * 9,
        out_specs=hbm,
        scratch_shapes=[
            pltpu.VMEM((8, 16, 4, W, 128), BF16),
            pltpu.VMEM((2, 4, 3, 3, C, 128), BF16),
            pltpu.VMEM((E, C), BF16),
            pltpu.VMEM((B, E), BF16),
            [pltpu.VMEM((C,), BF16)] * 4,
            pltpu.VMEM((5, 36, 4, 128, 128), BF16),
            pltpu.VMEM((36, 4, 256, 128), BF16),
            pltpu.VMEM((36, 4, 256, 128), BF16),
            pltpu.VMEM((8, 36, 256, 128), F32),
            pltpu.VMEM((8, 64, 4, 16, 128), F32),
            pltpu.VMEM((66, 6, 16, 128), F32),
            pltpu.VMEM((B, C), F32),
            pltpu.VMEM((16, 2, 8, 128), F32),
            pltpu.VMEM((16, 2, 8, 128), F32),
            pltpu.SemaphoreType.DMA((12,)),
            pltpu.SemaphoreType.DMA((11,)),
            pltpu.SemaphoreType.DMA((6,)),
            pltpu.SemaphoreType.DMA((12,)),
        ],
        compiler_params=pltpu.CompilerParams(
            vmem_limit_bytes=126 * 2 ** 20, disable_semaphore_checks=True),
        name="resblock",
    )(xt, t_emb, g1, be1, w1.transpose(2, 3, 0, 1), w_emb, g2, be2, w2.transpose(2, 3, 0, 1))
    return out.reshape(B, H, W, C).transpose(0, 3, 1, 2)
```
